```python
import os as _os
_os.environ.setdefault("JAX_PLATFORMS", "cpu")
import jax
import jax.numpy as jnp

def _softmax(x, axis=-1):
    return jax.nn.softmax(x, axis=axis)
def _gelu(x):
    return jax.nn.gelu(x, approximate=True)
def _silu(x):
    return jax.nn.silu(x)
def _sigmoid(x):
    return jax.nn.sigmoid(x)
def _layernorm(x, axis=-1, eps=1e-5):
    m = jnp.mean(x, axis=axis, keepdims=True)
    v = jnp.var(x, axis=axis, keepdims=True)
    return (x - m) / jnp.sqrt(v + eps)
def _scatter_add(tgt, idx, src, axis=0):
    return tgt.at[idx].add(src)
def _segment_sum(src, seg, n):
    return jax.ops.segment_sum(src, seg, n)
class _Rng:
    def __init__(self, key):
        self._k = key
    def _next(self):
        self._k, sub = jax.random.split(self._k)
        return sub
    def normal(self, shape):
        return jax.random.normal(self._next(), shape, dtype=jnp.bfloat16)
    def randint(self, lo, hi, shape):
        return jax.random.randint(self._next(), shape, lo, hi, dtype=jnp.int32)
    def uniform(self, shape, lo=0.0, hi=1.0):
        return jax.random.uniform(self._next(), shape, jnp.bfloat16, lo, hi)
    def permutation(self, n):
        return jax.random.permutation(self._next(), n)


kernel_name = 'concat_heads__spectral_gfnet__sliding_block__prompt'

def setup_inputs():
    _rng = _Rng(jax.random.key(int.from_bytes(__import__("os").urandom(4), "little")))
    _w = (lambda a: (lambda t: t.astype(jnp.bfloat16) if jnp.issubdtype(t.dtype, jnp.floating) else t)(jnp.asarray(a)))
    def _A_setup():
        B, S, D = 1, 2048, 640
        Df = D // 2 + 1
        return {
            "x": _w((lambda *s: _rng.normal(s) * 0.05)(B, S, D)),
            "w_r": _w((lambda *s: _rng.normal(s) * 0.4)(S, Df) * 0.02),
            "w_i": _w((lambda *s: _rng.normal(s) * 0.4)(S, Df) * 0.02),
        }
    _A_in = _A_setup()

    def _B_setup():
        B, S, D = 1, 2048, 640
        return {
            "x": _w((lambda *s: _rng.normal(s) * 0.2)(B, S, D)),
            "wqkv": _w((lambda *s: _rng.normal(s) * 0.2)(D, 3 * D)),
            "wo": _w((lambda *s: _rng.normal(s) * 0.05)(D, D)),
        }
    _B_in = _B_setup()

    return {
        "A_x": _A_in["x"],
        "A_w_r": _A_in["w_r"],
        "A_w_i": _A_in["w_i"],
        "B_x": _B_in["x"],
        "B_wqkv": _B_in["wqkv"],
        "B_wo": _B_in["wo"],
    }

def reference(A_x, A_w_r, A_w_i, B_x, B_wqkv, B_wo):
    def _A_ref(x, w_r, w_i):
        B, S, D = x.shape
        X = (lambda x, axes=(-2,-1): jnp.fft.rfft2(x.astype(jnp.float32), axes=axes))(x, axes=(-2, -1))
        W = w_r + 1j * w_i
        X = X * W
        y = (lambda x, s, axes=(-2,-1): jnp.fft.irfft2(x, s=s, axes=axes).astype(jnp.bfloat16))(X, (S, D), axes=(-2, -1))
        return y

    def _B_ref(x, wqkv, wo):
        B, S, D = x.shape
        H = 32; Dh = D // H; W = 256
        qkv = (lambda x, *d: x.transpose(*d))((x @ wqkv).reshape(B, S, 3, H, Dh), 2, 0, 3, 1, 4)
        q, k, v = qkv[0], qkv[1], qkv[2]
        scores = jnp.einsum("bhqd,bhkd->bhqk", q, k) * (Dh ** -0.5)
        idx = jnp.arange(S)
        mask = (idx[:, None] - idx[None, :] >= 0) & (idx[:, None] - idx[None, :] < W)
        scores = jnp.where(mask[None, None], scores, -1e9)
        p = _softmax(scores, axis=-1)
        o = jnp.einsum("bhqk,bhkd->bhqd", p, v)
        return (lambda x, *d: x.transpose(*d))(o, 0, 2, 1, 3).reshape(B, S, D) @ wo

    a = _A_ref(A_x, A_w_r, A_w_i)
    b = _B_ref(B_x, B_wqkv, B_wo)
    return jnp.concatenate([a, b], axis=-1)
```

```python
import numpy as np
import ml_dtypes
import jax
import jax.numpy as jnp
from jax import lax
import jax.experimental.pallas as pl
import jax.experimental.pallas.tpu as pltpu

bf = jnp.bfloat16
f32 = jnp.float32
S_ = 2048
D = 640
NB = 16
NH = 32
R = 32
QSCALE = float((20 ** -0.5) * np.log2(np.e))
NEG = -1e30


def _consts():
    n = np.arange(D)[:, None].astype(np.float64)
    c = lambda l: np.cos(2 * np.pi * n * l[None, :] / D)
    s = lambda l: -np.sin(2 * np.pi * n * l[None, :] / D)
    rd = np.concatenate([c(np.arange(0, 256)), c(np.arange(256, 320)), s(np.arange(256, 320)), s(np.arange(0, 256))], axis=1)
    rd[:, 384] = np.cos(np.pi * n[:, 0])
    perm = np.array([64 * ((r % 16) // 8) + 8 * (r // 16) + (r % 8) for r in range(128)])
    mf = np.zeros((R, 128, 128)); mi = np.zeros((R, 128, 128))
    k2 = np.arange(64)[:, None]; s2 = np.arange(64)[None, :]
    for k1 in range(R):
        ph = (s2 * (k1 + R * k2)) % S_
        M = np.exp(-2j * np.pi * ph / S_)
        mf[k1] = np.block([[M.real, -M.imag], [M.imag, M.real]])[perm][:, perm]
        A = M.conj().T * (2.0 / (S_ * D))
        mi[k1] = np.block([[A.real, -A.imag], [A.imag, A.real]])[perm][:, perm]
    b16 = ml_dtypes.bfloat16
    return rd.astype(np.float32).astype(b16), mf.astype(np.float32).astype(b16), mi.astype(np.float32).astype(b16)


RD_NP, MF_NP, MI_NP = _consts()


def _cmul_const(v, ang):
    re, im = v
    c, s = float(np.cos(ang)), float(np.sin(ang))
    eps = 1e-12
    if abs(s) < eps:
        return (re, im) if c > 0 else (-re, -im)
    if abs(c) < eps:
        return (-im, re) if s > 0 else (im, -re)
    if abs(abs(c) - abs(s)) < eps:
        h = abs(c)
        if c > 0 and s > 0: return ((re - im) * h, (re + im) * h)
        if c > 0 and s < 0: return ((re + im) * h, (im - re) * h)
        if c < 0 and s > 0: return ((re + im) * (-h), (re - im) * h)
        return ((im - re) * h, (re + im) * (-h))
    return (re * c - im * s, re * s + im * c)


def _fft(xs, sign):
    n = len(xs)
    if n == 1:
        return xs
    ev = _fft(xs[0::2], sign); od = _fft(xs[1::2], sign)
    out = [None] * n
    for k in range(n // 2):
        er, ei = ev[k]; orr, oi = od[k]
        if 4 * k == n:
            if sign < 0:
                out[k] = (er + oi, ei - orr); out[k + n // 2] = (er - oi, ei + orr)
            else:
                out[k] = (er - oi, ei + orr); out[k + n // 2] = (er + oi, ei - orr)
        else:
            tr, ti = _cmul_const((orr, oi), sign * 2 * np.pi * k / n)
            out[k] = (er + tr, ei + ti); out[k + n // 2] = (er - tr, ei - ti)
    return out


def _radix4(v, sign):
    (ar, ai), (br, bi), (cr, ci), (dr, di) = v
    s0r, s0i = ar + cr, ai + ci
    s1r, s1i = ar - cr, ai - ci
    s2r, s2i = br + dr, bi + di
    s3r, s3i = br - dr, bi - di
    o0 = (s0r + s2r, s0i + s2i)
    o2 = (s0r - s2r, s0i - s2i)
    if sign < 0:
        o1 = (s1r + s3i, s1i - s3r); o3 = (s1r - s3i, s1i + s3r)
    else:
        o1 = (s1r - s3i, s1i + s3r); o3 = (s1r + s3i, s1i - s3r)
    return [o0, o1, o2, o3]


def make_kernel(LAG=8, LAG1=2, TK=0, LA=1, DO_A=1, DO_B=1):
    def kernel(ax_h, wr_h, wi_h, bx_h, wqkv_h, wo_h, rd_h, mf_h, mi_h, out_h,
               xa, wr_v, wi_v, rd_v, mf_v, mi_v, X1, PR, PI, WR, WI, ZS, ya,
               xb, wqkv_v, wo_v, wT, KP, VT, QT, OT, OS, yb, sems, osem):
        cp = lambda s_, d_, i: pltpu.make_async_copy(s_, d_, sems.at[i])
        cp_rd = cp(rd_h, rd_v, 0)
        cp_xa = [cp(ax_h.at[pl.ds(512 * i, 512), :], xa.at[pl.ds(512 * i, 512), :], 1 + i) for i in range(4)]
        cp_wr = cp(wr_h, wr_v, 5); cp_wi = cp(wi_h, wi_v, 6)
        cp_mf = cp(mf_h, mf_v, 7); cp_mi = cp(mi_h, mi_v, 8)
        cp_w = cp(wqkv_h, wqkv_v, 9)
        cp_xb = [cp(bx_h.at[pl.ds(1024 * i, 1024), :], xb.at[pl.ds(1024 * i, 1024), :], 10 + i) for i in range(2)]
        cp_wo = cp(wo_h, wo_v, 12)
        cp_rd.start()
        for c_ in cp_xa: c_.start()

        sub8 = lax.broadcasted_iota(jnp.int32, (8, 128), 0)
        col8 = lax.broadcasted_iota(jnp.int32, (8, 128), 1)
        lane = lax.broadcasted_iota(jnp.int32, (128, 128), 1)
        lane16 = lax.broadcasted_iota(jnp.int32, (16, 128), 1)

        def init_pads():
            lane_k = lax.broadcasted_iota(jnp.int32, (128, 1024), 1)
            kpad = jnp.where((lane_k % 128) == 127, NEG, 0.0).astype(bf)
            KP[0] = kpad; KP[1] = kpad
            VT[0] = jnp.zeros((1024, 128), bf); VT[1] = jnp.zeros((1024, 128), bf)
            OT[...] = jnp.zeros(OT.shape, f32)

        def proj_k(b, xblk):
            kf = jnp.dot(xblk, wqkv_v[:, 640:1280], preferred_element_type=f32)
            for g in range(8):
                off = 80 * g; t = off // 128; sh = off % 128
                s0 = kf[:, 128 * t:128 * t + 128]
                if sh: s0 = pltpu.roll(s0, 128 - sh, 1)
                if sh + 80 > 128:
                    s1 = pltpu.roll(kf[:, 128 * (t + 1):128 * (t + 2)], 128 - sh, 1)
                    tile = jnp.where(lane < 128 - sh, s0, jnp.where(lane < 80, s1, 0.0))
                else:
                    tile = jnp.where(lane < 80, s0, 0.0)
                KP[b + 2, :, 128 * g:128 * g + 128] = tile.astype(bf)

        def proj_qv(b, xblk, slot):
            nt = lambda lo, n: lax.dot_general(wT[lo:lo + n, :], xblk, (((1,), (1,)), ((), ())), preferred_element_type=f32)
            QT[slot, 0:320, :] = nt(0, 320) * QSCALE
            QT[slot, 320:640, :] = nt(320, 320) * QSCALE
            vv = jnp.concatenate([nt(640, 320), nt(960, 320)], axis=0)
            cA = jnp.where(sub8 == 4, 1.0, 0.0).astype(f32)
            cB = jnp.where(sub8 == 0, 1.0, 0.0).astype(f32)
            z8 = jnp.zeros((8, 128), f32)
            for p in range(16):
                v = [vv[40 * p + 8 * i: 40 * p + 8 * i + 8] for i in range(5)]
                blk = jnp.concatenate([v[0], v[1], jnp.where(sub8 < 4, v[2], cA), z8,
                                       jnp.where(sub8 >= 4, v[2], cB), v[3], v[4], z8], axis=0)
                VT[b + 2, 64 * p:64 * p + 64, :] = blk.astype(bf)

        def build_w(h, slot):
            g, i = h // 4, h % 4
            a = (20 * i) // 16
            q = QT[slot, g * 80 + 16 * a: g * 80 + 16 * a + 32, :]
            r = lax.broadcasted_iota(jnp.int32, (32, 128), 0) + 16 * a
            qm = jnp.where((r >= 20 * i) & (r < 20 * i + 20), q, 0.0)
            parts = []
            if a > 0: parts.append(jnp.zeros((16 * a, 128), f32))
            parts.append(qm)
            parts.append(jnp.zeros((120 - 16 * a - 32, 128), f32))
            parts.append(jnp.where(sub8 == 7, 1.0, 0.0).astype(f32))
            return jnp.concatenate(parts, axis=0).astype(bf)

        def qk_dot(b, h, slot):
            g = h // 4
            w = build_w(h, slot)
            lo, hi = g * 128, (g + 1) * 128
            pieces = []
            for a in range(8):
                pieces.append(KP[b, 16 * a:16 * a + 16, lo:hi])
                pieces.append(KP[b + 2, 16 * a:16 * a + 16, lo:hi])
            pieces.append(KP[b + 1, :, lo:hi])
            kt = jnp.concatenate(pieces, axis=0)
            return jnp.dot(kt, w, preferred_element_type=f32)

        def max_stage(si):
            mx = None; scs = []
            for a in range(16):
                o_ = (a // 2) * 32 + (a % 2) * 8
                first = si[o_: o_ + 8]
                last = si[o_ + 16: o_ + 24]
                sc = jnp.where(sub8 + 8 * a > col8, first, last)
                scs.append(sc)
                mx = sc if mx is None else jnp.maximum(mx, sc)
            sm = si[256:384]
            for a in range(16):
                mx = jnp.maximum(mx, sm[8 * a:8 * a + 8])
            mx = jnp.max(mx, axis=0, keepdims=True)
            return (jnp.concatenate(scs, axis=0), sm, mx)

        def exp_pv(b, h, st):
            sc, sm, m = st
            row = lax.broadcasted_iota(jnp.int32, (128, 128), 0)
            pc = jnp.exp2(sc - m)
            pm = jnp.exp2(sm - m)
            msk = row > lane
            pu = jnp.where(msk, pc, 0.0)
            pl_ = jnp.where(msk, 0.0, pc)
            pall = jnp.concatenate([pu, pm, pl_], axis=0).astype(bf)
            vt = jnp.concatenate([VT[b + t, 32 * h:32 * h + 32, :] for t in range(3)], axis=1)
            o = jnp.dot(vt, pall, preferred_element_type=f32)
            l = o[20:21, :] if h % 2 == 0 else o[0:1, :]
            r = pltpu.reciprocal(l, approx=False)
            return o[0:24] * r

        def fin_o():
            for kt in range(5):
                OS[:, 128 * kt:128 * kt + 128] = OT[128 * kt:128 * kt + 128, :].T.astype(bf)

        def outproj(bprev):
            y = jnp.dot(OS[...], wo_v[...], preferred_element_type=f32)
            yb[pl.ds(pl.multiple_of(bprev * 128, 128), 128), :] = y.astype(bf)

        def out_copy(bb):
            return pltpu.make_async_copy(yb.at[pl.ds(pl.multiple_of(bb * 128, 128), 128), :],
                                         out_h.at[pl.ds(pl.multiple_of(bb * 128, 128), 128), pl.ds(640, 640)], osem.at[0])

        def rows_of(a, b):
            return 64 * (a + 4 * b)

        def dfwd_dot(c, n):
            rs = pl.ds(512 * c, 512)
            X1[rs, 128 * n:128 * n + 128] = jnp.dot(xa[rs, :], rd_v[:, 128 * n:128 * n + 128], preferred_element_type=f32)

        def fwd_fft_unit(a, p, j):
            xs = []
            for b in range(8):
                r = pl.ds(rows_of(a, b) + 16 * j, 16)
                if p == 0:
                    re = X1[r, 0:128]; im = jnp.where(lane16 == 0, 0.0, X1[r, 384:512])
                elif p == 1:
                    re = X1[r, 128:256]; im = X1[r, 512:640]
                else:
                    m = X1[r, 256:384]
                    re = jnp.where(lane16 < 64, m, jnp.where(lane16 == 64, pltpu.roll(X1[r, 384:512], 64, 1), 0.0))
                    im = jnp.where(lane16 < 64, pltpu.roll(m, 64, 1), 0.0)
                xs.append((re, im))
            ys = _fft(xs, -1)
            for kp in range(8):
                y = _cmul_const(ys[kp], -2 * np.pi * a * kp / 32)
                PR[p, a * 8 + kp, 16 * j:16 * j + 16, :] = y[0]
                PI[p, a * 8 + kp, 16 * j:16 * j + 16, :] = y[1]

        def wprep(c):
            for src, dst in ((wr_v, WR), (wi_v, WI)):
                cs = slice(128 * c, 128 * c + 128)
                w0 = src[0:128, cs].astype(f32).T
                w0 = jnp.where(lane == 0, 0.5 * w0, w0)
                w1 = src[128:256, cs].astype(f32).T
                w2 = jnp.concatenate([src[256:321, cs].astype(f32), jnp.zeros((63, 128), f32)], axis=0).T
                w2 = jnp.where(lane == 64, 0.5 * w2, w2)
                for p, w in enumerate((w0, w1, w2)):
                    for q in range(4):
                        dst[p, pl.ds(33 * (4 * c + q), 32), :] = w[32 * q:32 * q + 32]

        def pre(kp, p):
            tiles = [[] for _ in range(4)]
            for g in range(8):
                v = [(PR[p, a * 8 + kp, 8 * g:8 * g + 8, :], PI[p, a * 8 + kp, 8 * g:8 * g + 8, :]) for a in range(4)]
                ts = _radix4(v, -1)
                for kk in range(4): tiles[kk] += [ts[kk][0], ts[kk][1]]
            return [jnp.concatenate(t, axis=0).astype(bf) for t in tiles]

        def fwd(kp, p, ts):
            return [jnp.dot(mf_v[kp + 8 * kk], ts[kk], preferred_element_type=f32) for kk in range(4)]

        def mid(kp, p, xs):
            outs = []
            for kk in range(4):
                k1 = kp + 8 * kk
                x = xs[kk]
                ys = []
                for g in range(8):
                    xr, xi = x[16 * g:16 * g + 8], x[16 * g + 8:16 * g + 16]
                    wr = WR[p, pl.ds(k1 + 33 * 8 * g, 8, stride=33), :]
                    wi = WI[p, pl.ds(k1 + 33 * 8 * g, 8, stride=33), :]
                    ys += [xr * wr - xi * wi, xr * wi + xi * wr]
                y = jnp.concatenate(ys, axis=0).astype(bf)
                outs.append(jnp.dot(mi_v[k1], y, preferred_element_type=f32))
            return outs

        def post(kp, p, outs):
            for g in range(8):
                v = [(o[16 * g:16 * g + 8], o[16 * g + 8:16 * g + 16]) for o in outs]
                r = _radix4(v, +1)
                for a in range(4):
                    PR[p, a * 8 + kp, 8 * g:8 * g + 8, :] = r[a][0]
                    PI[p, a * 8 + kp, 8 * g:8 * g + 8, :] = r[a][1]

        def inv_fft_unit(a, p, j):
            xs = []
            for kp in range(8):
                v = (PR[p, a * 8 + kp, 16 * j:16 * j + 16, :], PI[p, a * 8 + kp, 16 * j:16 * j + 16, :])
                xs.append(_cmul_const(v, 2 * np.pi * a * kp / 32))
            zs = _fft(xs, +1)
            for b in range(8):
                r = pl.ds(512 * a + 64 * b + 16 * j, 16)
                zr, zi = zs[b]
                if p == 2:
                    ZS[r, 256:384] = jnp.where(lane16 < 64, zr, pltpu.roll(zi, 64, 1)).astype(bf)
                    ZS[r, 384:512] = pltpu.roll(zr, 64, 1).astype(bf)
                elif p == 0:
                    ZS[r, 0:128] = zr.astype(bf)
                    ZS[r, 384:512] = jnp.where(lane16 == 0, ZS[r, 384:512].astype(f32), zi).astype(bf)
                else:
                    ZS[r, 128:256] = zr.astype(bf)
                    ZS[r, 512:640] = zi.astype(bf)

        def dinv_dot(a, n):
            y = lax.dot_general(ZS[pl.ds(512 * a, 512), :], rd_v[128 * n:128 * n + 128, :], (((1,), (1,)), ((), ())), preferred_element_type=f32)
            yb_ = y.astype(bf)
            for b in range(8):
                ya[pl.ds(rows_of(a, b), 64), 128 * n:128 * n + 128] = yb_[64 * b:64 * b + 64]

        a_out = pltpu.make_async_copy(ya, out_h.at[:, pl.ds(0, 640)], osem.at[1])
        fft_units = [(a, j) for a in range(4) for j in range(4)]

        def mxu_stage(p, extra):
            st = {}
            for t in range(8 + LA + 1):
                if t < 8: st[t] = ('f', fwd(t, p, pre(t, p)))
                u = t - LA
                if 0 <= u < 8: st[u] = ('m', mid(u, p, st[u][1]))
                u = t - LA - 1
                if 0 <= u < 8: post(u, p, st.pop(u)[1])
                if t < 8: extra(t)

        init_pads()
        cp_rd.wait()
        cp_xa[0].wait()
        for c_ in (cp_wr, cp_wi, cp_mf, cp_mi, cp_w, cp_xb[0], cp_wo, cp_xb[1]): c_.start()
        for c in range(4):
            if c > 0: cp_xa[c].wait()
            dfwd_dot(c, 2); dfwd_dot(c, 3)
        cp_wr.wait(); cp_wi.wait()
        for c in range(4):
            dfwd_dot(c, 0)
            for (a, j) in fft_units[4 * c:4 * c + 4]: fwd_fft_unit(a, 2, j)
            for q in range(2 * c, 2 * c + 2): wprep(q)
        cp_w.wait()
        for i in range(8):
            dfwd_dot(i // 2, (1, 4)[i % 2])
            for (a, j) in fft_units[2 * i:2 * i + 2]: fwd_fft_unit(a, 0, j)
            wprep(8 + i)
            if i % 4 != 3:
                pass
            if i < 5:
                wT[128 * i:128 * i + 128, :] = wqkv_v[:, 128 * i:128 * i + 128].T
                wT[640 + 128 * i:640 + 128 * i + 128, :] = wqkv_v[:, 1280 + 128 * i:1280 + 128 * i + 128].T
        cp_mf.wait(); cp_mi.wait()
        mxu_stage(2, lambda t: [fwd_fft_unit(a, 1, j) for (a, j) in fft_units[2 * t:2 * t + 2]])
        mxu_stage(0, lambda t: [inv_fft_unit(a, 2, j) for (a, j) in fft_units[2 * t:2 * t + 2]])
        mxu_stage(1, lambda t: [inv_fft_unit(a, 0, j) for (a, j) in fft_units[2 * t:2 * t + 2]])
        cp_xb[0].wait()
        x0 = xb[0:128, :]
        for j in range(4): inv_fft_unit(0, 1, j)
        proj_k(0, x0)
        for a in range(4):
            for n in range(5):
                dinv_dot(a, n)
                if a + 1 < 4 and n < 4: inv_fft_unit(a + 1, 1, n)
        proj_qv(0, x0, 0)
        a_out.start()
        cp_wo.wait()

        def body(b, carry):
            slot = b % 2
            bn = jnp.minimum(b + 1, NB - 1)
            bp = jnp.maximum(b - 1, 0)

            @pl.when(bn == 8)
            def _():
                cp_xb[1].wait()
            dots = {}; sts = {}; outs = {}
            for t in range(NH + LAG):
                if t < NH: dots[t] = qk_dot(b, t, slot)
                if t == 0: fin_o()
                if t == 2: outproj(bp)
                if 0 <= t - LAG1 < NH: sts[t - LAG1] = max_stage(dots.pop(t - LAG1))
                if t == NH + TK:
                    xn = xb[pl.ds(pl.multiple_of(bn * 128, 128), 128), :]
                    proj_k(bn, xn)
                if 0 <= t - LAG < NH:
                    h = t - LAG
                    outs[h] = exp_pv(b, h, sts.pop(h))
                    if h % 2 == 1:
                        A = outs.pop(h - 1); B = outs.pop(h)
                        p = h // 2
                        OT[40 * p:40 * p + 40, :] = jnp.concatenate([A[0:16], jnp.where(sub8 < 4, A[16:24], B[0:8]), B[8:24]], axis=0)
            proj_qv(bn, xn, 1 - slot)

            @pl.when(b > 0)
            def _():
                out_copy(bp).start()
            return carry
        lax.fori_loop(0, NB, body, 0)
        fin_o()
        outproj(NB - 1)
        out_copy(NB - 1).start()
        a_out.wait()
        for i in range(NB):
            out_copy(i).wait()
    return kernel


def run(A_x, A_w_r, A_w_i, B_x, B_wqkv, B_wo, **kw):
    kernel = make_kernel(**kw)
    hbm = pl.BlockSpec(memory_space=pltpu.HBM)
    V = pltpu.VMEM
    out = pl.pallas_call(
        kernel,
        out_shape=jax.ShapeDtypeStruct((S_, 2 * D), bf),
        in_specs=[hbm] * 9, out_specs=hbm,
        scratch_shapes=[
            V((S_, D), bf), V((321, S_), bf), V((321, S_), bf),
            V((D, D), bf), V((R, 128, 128), bf), V((R, 128, 128), bf),
            V((S_, D), f32),
            V((3, 32, 64, 128), f32), V((3, 32, 64, 128), f32),
            V((3, 2112, 128), f32), V((3, 2112, 128), f32),
            V((S_, D), bf), V((S_, D), bf),
            V((S_, D), bf), V((D, 3 * D), bf), V((D, D), bf), V((2 * D, D), bf),
            V((NB + 2, 128, 1024), bf), V((NB + 2, 1024, 128), bf),
            V((2, D, 128), f32), V((D, 128), f32), V((128, D), bf), V((S_, D), bf),
            pltpu.SemaphoreType.DMA((13,)), pltpu.SemaphoreType.DMA((2,)),
        ],
        compiler_params=pltpu.CompilerParams(vmem_limit_bytes=110 * 2**20),
        name='fused',
    )(A_x.reshape(S_, D), A_w_r.T, A_w_i.T, B_x.reshape(S_, D), B_wqkv, B_wo,
      jnp.asarray(RD_NP), jnp.asarray(MF_NP), jnp.asarray(MI_NP))
    return out.reshape(1, S_, 2 * D)


@jax.jit
def pallas_concat_heads__spectral_gfnet__sliding_block__prompt_kernel(
    A_x: jax.Array,
    A_w_r: jax.Array,
    A_w_i: jax.Array,
    B_x: jax.Array,
    B_wqkv: jax.Array,
    B_wo: jax.Array,
):
    return run(A_x, A_w_r, A_w_i, B_x, B_wqkv, B_wo)
```

```python
import numpy as np
import ml_dtypes
import jax
import jax.numpy as jnp
from jax import lax
import jax.experimental.pallas as pl
import jax.experimental.pallas.tpu as pltpu

bf = jnp.bfloat16
f32 = jnp.float32
S_ = 2048
D = 640
NB = 16
NH = 32
R = 32
QSCALE = float((20 ** -0.5) * np.log2(np.e))
NEG = -1e30


def _consts():
    n2 = np.arange(128)[:, None].astype(np.float64)

    m_ = np.arange(32)

    def gmat(r1, r2):
        l = np.concatenate([r1 + 10 * m_, r1 + 5 + 10 * m_, r2 + 10 * m_, r2 + 5 + 10 * m_]).astype(np.float64)[None, :]
        c = np.cos(2 * np.pi * n2 * l / D); s = np.sin(2 * np.pi * n2 * l / D)
        sg = np.concatenate([np.ones(64), -np.ones(64)])[None, :]
        return np.block([[c, -s], [sg * s, sg * c]])
    g = np.zeros((3, 256, 256))
    g[0] = gmat(1, 4)
    g[1] = gmat(2, 3)
    l0 = np.concatenate([10 * m_, 5 + 10 * m_]).astype(np.float64)[None, :]
    g0 = np.concatenate([np.cos(2 * np.pi * n2 * l0 / D), -np.sin(2 * np.pi * n2 * l0 / D)], axis=1)
    g0[:, 64] = np.cos(np.pi * n2[:, 0])
    g[2, :128, :128] = g0
    perm_out = np.array([64 * ((r % 16) // 8) + 8 * (r // 16) + (r % 8) for r in range(128)])
    perm_in = np.array([64 * (r % 2) + 8 * (r // 16) + ((r % 16) // 2) for r in range(128)])
    pre = np.array([16 * (r // 16) + 2 * (r % 8) + ((r % 16) // 8) for r in range(128)])
    k2 = np.arange(64)[:, None]; s2 = np.arange(64)[None, :]
    F = np.exp(-2j * np.pi * ((s2 * k2) % 64) / 64)
    e1 = np.block([[F.real, -F.imag], [F.imag, F.real]])
    e2 = np.block([[-F.imag, -F.real], [F.real, -F.imag]])
    rows_f = perm_out[pre]
    cols_i = perm_out[pre]
    E = np.stack([e1[rows_f][:, perm_in], e2[rows_f][:, perm_in], e1[perm_in][:, cols_i], e2[perm_in][:, cols_i]])
    s2f = perm_in % 64; s2i = cols_i % 64
    k1 = np.arange(R)[:, None]
    CS = np.stack([np.cos(2 * np.pi * ((k1 * s2f[None, :]) % S_) / S_), -np.sin(2 * np.pi * ((k1 * s2f[None, :]) % S_) / S_),
                   np.cos(2 * np.pi * ((k1 * s2i[None, :]) % S_) / S_), -np.sin(2 * np.pi * ((k1 * s2i[None, :]) % S_) / S_)])
    b16 = ml_dtypes.bfloat16
    return g.astype(np.float32).astype(b16), E.astype(np.float32), CS.astype(np.float32)


RD_NP, E_NP, CS_NP = _consts()
SIG = float(2.0 / (S_ * D))
C1, C2 = float(np.cos(2 * np.pi / 5)), float(np.cos(4 * np.pi / 5))
S1, S2 = float(np.sin(2 * np.pi / 5)), float(np.sin(4 * np.pi / 5))


def _radix5_fwd(x):
    t1, t2 = x[1] + x[4], x[2] + x[3]
    t3, t4 = x[1] - x[4], x[2] - x[3]
    a0 = x[0] + t1 + t2
    a1 = x[0] + C1 * t1 + C2 * t2
    a2 = x[0] + C2 * t1 + C1 * t2
    b1 = -(S1 * t3 + S2 * t4)
    b2 = S1 * t4 - S2 * t3
    return [a0, a1, b1, a2, b2]


def _radix5_inv(q0, q1r, q1i, q2r, q2i):
    q0s = SIG * q0
    t1 = q0s + (SIG * C1) * q1r + (SIG * C2) * q2r
    t2 = q0s + (SIG * C2) * q1r + (SIG * C1) * q2r
    u1 = (SIG * S1) * q1i + (SIG * S2) * q2i
    u2 = (SIG * S2) * q1i - (SIG * S1) * q2i
    return [SIG * (q0 + q1r + q2r), t1 - u1, t2 - u2, t2 + u2, t1 + u1]


def _pack_rows_u32(m):
    u = m.view(np.uint16).astype(np.uint32)
    return (u[..., 0::2, :] | (u[..., 1::2, :] << 16)).astype(np.uint32)


RD_U32 = _pack_rows_u32(RD_NP)


def _cmul_const(v, ang):
    re, im = v
    c, s = float(np.cos(ang)), float(np.sin(ang))
    eps = 1e-12
    if abs(s) < eps:
        return (re, im) if c > 0 else (-re, -im)
    if abs(c) < eps:
        return (-im, re) if s > 0 else (im, -re)
    if abs(abs(c) - abs(s)) < eps:
        h = abs(c)
        if c > 0 and s > 0: return ((re - im) * h, (re + im) * h)
        if c > 0 and s < 0: return ((re + im) * h, (im - re) * h)
        if c < 0 and s > 0: return ((re + im) * (-h), (re - im) * h)
        return ((im - re) * h, (re + im) * (-h))
    return (re * c - im * s, re * s + im * c)


def _fft(xs, sign):
    n = len(xs)
    if n == 1:
        return xs
    ev = _fft(xs[0::2], sign); od = _fft(xs[1::2], sign)
    out = [None] * n
    for k in range(n // 2):
        er, ei = ev[k]; orr, oi = od[k]
        if 4 * k == n:
            if sign < 0:
                out[k] = (er + oi, ei - orr); out[k + n // 2] = (er - oi, ei + orr)
            else:
                out[k] = (er - oi, ei + orr); out[k + n // 2] = (er + oi, ei - orr)
        else:
            tr, ti = _cmul_const((orr, oi), sign * 2 * np.pi * k / n)
            out[k] = (er + tr, ei + ti); out[k + n // 2] = (er - tr, ei - ti)
    return out


def _radix4(v, sign):
    (ar, ai), (br, bi), (cr, ci), (dr, di) = v
    s0r, s0i = ar + cr, ai + ci
    s1r, s1i = ar - cr, ai - ci
    s2r, s2i = br + dr, bi + di
    s3r, s3i = br - dr, bi - di
    o0 = (s0r + s2r, s0i + s2i)
    o2 = (s0r - s2r, s0i - s2i)
    if sign < 0:
        o1 = (s1r + s3i, s1i - s3r); o3 = (s1r - s3i, s1i + s3r)
    else:
        o1 = (s1r - s3i, s1i + s3r); o3 = (s1r + s3i, s1i - s3r)
    return [o0, o1, o2, o3]


def make_kernel(LAG=8, LAG1=2, TK=0, LA=2, WU0=11, NWU=5, MB0=8, PK=0, PQ=13, UNR=1, LQ=1, ORD=1, LI=1, TO=2, TF=0, TQ=-1):
    def kernel(ax_h, wr_h, wi_h, bx_h, wqkv_h, wo_h, rd_h, e_h, cs_h, out_h,
               xa, wr_v, wi_v, rd_v, mf_v, mi_v, e_v, cs_v, wr_n, wi_n, PR, PI, WW, Y, TS, YS, ZS, XL,
               xb, wqkv_v, wo_v, wT, KP, VT, QT, OT, OS, sems, osem):
        cp = lambda s_, d_, i: pltpu.make_async_copy(s_, d_, sems.at[i])
        cp_rd = cp(rd_h, rd_v, 0)
        cp_xa = [cp(ax_h.at[:, i].bitcast(jnp.uint32), xa.at[i], 1 + i) for i in range(4)]
        wsl = lambda h_, c: h_.at[pl.ds(0, 320), pl.ds(128 * c, 128)].bitcast(jnp.uint32)
        cp_wg = [[cp(wsl(h_, c), v_.at[c], 5 + g_) for c in range(8 * g_, 8 * g_ + 8) for (h_, v_) in ((wr_h, wr_v), (wi_h, wi_v))]
                 for g_ in range(2)]
        cp_wg[0] += [cp(wr_h.at[pl.ds(320, 1), :], wr_n, 5), cp(wi_h.at[pl.ds(320, 1), :], wi_n, 5)]
        cp_e = [cp(e_h, e_v, 7), cp(cs_h, cs_v, 7)]
        cp_w = cp(wqkv_h.bitcast(jnp.uint32), wqkv_v, 9)
        cp_xb = [cp(bx_h.at[pl.ds(0, 256), :].bitcast(jnp.uint32), xb.at[pl.ds(0, 128), :], 9),
                 cp(bx_h.at[pl.ds(256, 1792), :].bitcast(jnp.uint32), xb.at[pl.ds(128, 896), :], 10)]
        cp_wo = cp(wo_h.bitcast(jnp.uint32), wo_v, 10)
        cp_rd.start()
        cp_xa[0].start()

        tb = lambda v: pltpu.bitcast(v, bf)
        pk2 = lambda a_, b_: pltpu.pack_elementwise([a_, b_], packed_dtype=bf)
        sub8 = lax.broadcasted_iota(jnp.int32, (8, 128), 0)
        col8 = lax.broadcasted_iota(jnp.int32, (8, 128), 1)
        lane = lax.broadcasted_iota(jnp.int32, (128, 128), 1)
        lane16 = lax.broadcasted_iota(jnp.int32, (16, 128), 1)

        def init_pads():
            lane_k = lax.broadcasted_iota(jnp.int32, (128, 1024), 1)
            kpad = jnp.where((lane_k % 128) == 127, NEG, 0.0).astype(bf)
            KP[0] = kpad; KP[1] = kpad
            VT[0] = jnp.zeros((1024, 128), bf); VT[1] = jnp.zeros((1024, 128), bf)
            OT[...] = jnp.zeros(OT.shape, f32)

        def proj_k(b, xblk):
            kf = jnp.dot(xblk, tb(wqkv_v[:, 640:1280]), preferred_element_type=f32)
            for g in range(8):
                off = 80 * g; t = off // 128; sh = off % 128
                s0 = kf[:, 128 * t:128 * t + 128]
                if sh: s0 = pltpu.roll(s0, 128 - sh, 1)
                if sh + 80 > 128:
                    s1 = pltpu.roll(kf[:, 128 * (t + 1):128 * (t + 2)], 128 - sh, 1)
                    tile = jnp.where(lane < 128 - sh, s0, jnp.where(lane < 80, s1, 0.0))
                else:
                    tile = jnp.where(lane < 80, s0, 0.0)
                KP[b + 2, :, 128 * g:128 * g + 128] = tile.astype(bf)

        def proj_qv(b, xblk, slot):
            nt = lambda lo, n: lax.dot_general(wT[lo:lo + n, :], xblk, (((1,), (1,)), ((), ())), preferred_element_type=f32)
            QT[slot, 0:320, :] = nt(0, 320) * QSCALE
            QT[slot, 320:640, :] = nt(320, 320) * QSCALE
            vv = jnp.concatenate([nt(640, 320), nt(960, 320)], axis=0)
            cA = jnp.where(sub8 == 4, 1.0, 0.0).astype(f32)
            cB = jnp.where(sub8 == 0, 1.0, 0.0).astype(f32)
            z8 = jnp.zeros((8, 128), f32)
            for p in range(16):
                v = [vv[40 * p + 8 * i: 40 * p + 8 * i + 8] for i in range(5)]
                blk = jnp.concatenate([v[0], v[1], jnp.where(sub8 < 4, v[2], cA), z8,
                                       jnp.where(sub8 >= 4, v[2], cB), v[3], v[4], z8], axis=0)
                VT[b + 2, 64 * p:64 * p + 64, :] = blk.astype(bf)

        def build_w(h, slot):
            g, i = h // 4, h % 4
            a = (20 * i) // 16
            q = QT[slot, g * 80 + 16 * a: g * 80 + 16 * a + 32, :]
            r = lax.broadcasted_iota(jnp.int32, (32, 128), 0) + 16 * a
            qm = jnp.where((r >= 20 * i) & (r < 20 * i + 20), q, 0.0)
            parts = []
            if a > 0: parts.append(jnp.zeros((16 * a, 128), f32))
            parts.append(qm)
            parts.append(jnp.zeros((120 - 16 * a - 32, 128), f32))
            parts.append(jnp.where(sub8 == 7, 1.0, 0.0).astype(f32))
            return jnp.concatenate(parts, axis=0).astype(bf)

        lane64 = lax.broadcasted_iota(jnp.int32, (64, 128), 1)

        def build_wd(h, slot):
            g, i = h // 4, h % 4
            a = (20 * i) // 16
            q = QT[slot, g * 80 + 16 * a: g * 80 + 16 * a + 32, :]
            r = lax.broadcasted_iota(jnp.int32, (32, 128), 0) + 16 * a
            c = lax.broadcasted_iota(jnp.int32, (32, 128), 1)
            qf = jnp.where((r >= 20 * i) & (r < 20 * i + 20) & (c < 64), q, 0.0)
            o_ = (20 * i) % 8
            q2 = QT[slot, g * 80 + 20 * i - o_: g * 80 + 20 * i - o_ + 24, :]
            r2 = lax.broadcasted_iota(jnp.int32, (24, 128), 0)
            c2 = lax.broadcasted_iota(jnp.int32, (24, 128), 1)
            ql = jnp.where((r2 >= o_) & (r2 < o_ + 20) & (c2 >= 64), q2, 0.0)
            parts = []
            if a > 0: parts.append(jnp.zeros((16 * a, 128), f32))
            parts.append(qf)
            if 80 - 16 * a - 32 > 0: parts.append(jnp.zeros((80 - 16 * a - 32, 128), f32))
            parts.append(ql)
            parts.append(jnp.zeros((16, 128), f32))
            parts.append(jnp.where((sub8 == 7) & (col8 < 64), 1.0, 0.0).astype(f32))
            return jnp.concatenate(parts, axis=0).astype(bf)

        def qk_dot(b, h, slot):
            g, i = h // 4, h % 4
            w = build_w(h, slot)
            lo, hi = g * 128, (g + 1) * 128
            kt = jnp.concatenate([KP[b + 2, 0:64, lo:hi], KP[b, 64:128, lo:hi], KP[b + 1, :, lo:hi]], axis=0)
            main = jnp.dot(kt, w, preferred_element_type=f32)
            sh = 80 + (20 * i) % 8 - 20 * i
            rl = pltpu.roll(KP[b + 2, 64:128, lo:hi], sh, 1)
            ld = jnp.where((lane64 >= 80) & (lane64 < 104), rl, KP[b, 0:64, lo:hi])
            diag = jnp.dot(ld, build_wd(h, slot), preferred_element_type=f32)
            return main, diag

        def max_stage(sd):
            si, dg = sd
            mx = None; scs = []
            for a in range(16):
                if a < 8: first, last = dg[8 * a:8 * a + 8], si[8 * a:8 * a + 8]
                else: first, last = si[8 * a:8 * a + 8], dg[8 * a - 64:8 * a - 56]
                sc = jnp.where(sub8 + 8 * a > col8, first, last)
                scs.append(sc)
                mx = sc if mx is None else jnp.maximum(mx, sc)
            sm = si[128:256]
            for a in range(16):
                mx = jnp.maximum(mx, sm[8 * a:8 * a + 8])
            mx = jnp.max(mx, axis=0, keepdims=True)
            return (jnp.concatenate(scs, axis=0), sm, mx)

        def exp_pv(b, h, st):
            sc, sm, m = st
            row = lax.broadcasted_iota(jnp.int32, (128, 128), 0)
            pc = jnp.exp2(sc - m)
            pm = jnp.exp2(sm - m)
            msk = row > lane
            pu = jnp.where(msk, pc, 0.0)
            pl_ = jnp.where(msk, 0.0, pc)
            pall = jnp.concatenate([pu, pm, pl_], axis=0).astype(bf)
            vt = jnp.concatenate([VT[b + t, 32 * h:32 * h + 32, :] for t in range(3)], axis=1)
            o = jnp.dot(vt, pall, preferred_element_type=f32)
            l = o[20:21, :] if h % 2 == 0 else o[0:1, :]
            r = pltpu.reciprocal(l, approx=False)
            return o[0:24] * r

        def fin_o():
            for kt in range(5):
                OS[:, 128 * kt:128 * kt + 128] = OT[128 * kt:128 * kt + 128, :].T.astype(bf)

        def outproj(bprev):
            y = jnp.dot(OS[...], tb(wo_v[...]), preferred_element_type=f32)
            Y[1, pl.ds(pl.multiple_of(bprev * 128, 128), 128), :] = y.astype(bf)

        def out_copy(bb, half):
            return pltpu.make_async_copy(Y.at[half, pl.ds(pl.multiple_of(bb * 128, 128), 128), :],
                                         out_h.at[pl.ds(pl.multiple_of(bb * 128, 128), 128), pl.ds(pl.multiple_of(640 * half, 128), 640)], osem.at[0])

        def rows_of(a, b):
            return 64 * (a + 4 * b)

        xau = xa
        upk = lambda w_, i_: pltpu.unpack_elementwise(w_, index=i_, packed_dtype=bf, unpacked_dtype=f32)

        def r5_fwd(u, bs):
            a, j = fft_units[u]
            for b in bs:
                ws = [xau[a, b, 8 * j:8 * j + 8, 128 * t:128 * t + 128] for t in range(5)]
                oe = _radix5_fwd([upk(w_, 0) for w_ in ws])
                oo = _radix5_fwd([upk(w_, 1) for w_ in ws])
                for t in range(5):
                    XL[u % 3, 8 * b:8 * b + 8, 128 * t:128 * t + 128] = pk2(oe[t], oo[t])

        def dfwd_dot(u, n):
            if n == 0:
                r_ = jnp.dot(tb(XL[u % 3, :, 128:384]), tb(rd_v[0]), preferred_element_type=f32)
                return (r_[:, 0:128], r_[:, 128:256])
            if n == 1:
                r_ = jnp.dot(tb(XL[u % 3, :, 384:640]), tb(rd_v[1]), preferred_element_type=f32)
                return (r_[:, 0:128], r_[:, 128:256])
            return jnp.dot(tb(XL[u % 3, :, 0:128]), tb(rd_v[2, 0:64, 0:128]), preferred_element_type=f32)

        lane8 = col8

        def fwd_fft_unit(a, p, j, t):
          for hh in range(2):
            xs = []
            for b in range(8):
                r = slice(16 * b + 8 * hh, 16 * b + 8 * hh + 8)
                if p < 2:
                    re = t[0][r]; im = t[1][r]
                else:
                    m = t[r]
                    re = jnp.where(lane8 <= 64, m, 0.0)
                    im = jnp.where((lane8 >= 1) & (lane8 < 64), pltpu.roll(m, 64, 1), 0.0)
                xs.append((re, im))
            ys = _fft(xs, -1)
            for kp in range(8):
                y = _cmul_const(ys[kp], -2 * np.pi * a * kp / 32)
                rr = slice(16 * j + 8 * hh, 16 * j + 8 * hh + 8)
                PR[p, a * 8 + kp, rr, :] = y[0]
                PI[p, a * 8 + kp, rr, :] = y[1]

        wru = wr_v; wiu = wi_v

        def wprep1(c, p):
            def rows(rho):
                sl = pl.ds(rho // 2, 32, stride=5)
                a_ = upk(wru[c, sl, :], rho % 2); b_ = upk(wiu[c, sl, :], rho % 2)
                if rho == 0:
                    r32 = lax.broadcasted_iota(jnp.int32, (32, 128), 0)
                    a_ = jnp.where(r32 == 0, 0.5 * a_, a_); b_ = jnp.where(r32 == 0, 0.5 * b_, b_)
                return pk2(a_, b_)
            if p < 2:
                r1, r2 = (1, 4) if p == 0 else (2, 3)
                w = jnp.concatenate([rows(r1), rows(r1 + 5), rows(r2), rows(r2 + 5)], axis=0)
            else:
                a_ = jnp.where(sub8 == 0, 0.5 * jnp.broadcast_to(wr_n[0:1, 128 * c:128 * c + 128].astype(f32), (8, 128)), 0.0)
                b_ = jnp.where(sub8 == 0, 0.5 * jnp.broadcast_to(wi_n[0:1, 128 * c:128 * c + 128].astype(f32), (8, 128)), 0.0)
                w = jnp.concatenate([rows(0), rows(5), pk2(a_, b_), jnp.zeros((56, 128), jnp.uint32)], axis=0)
            w = w.T
            for q in range(4):
                WW[p, pl.ds(33 * (4 * c + q), 32), :] = w[32 * q:32 * q + 32]

        def mbuild(k1):
            cf = jnp.broadcast_to(cs_v[0, k1:k1 + 1, :], (8, 128)); sf = jnp.broadcast_to(cs_v[1, k1:k1 + 1, :], (8, 128))
            for v in range(8):
                lo = e_v[0, 16 * v:16 * v + 8, :] * cf + e_v[1, 16 * v:16 * v + 8, :] * sf
                hi = e_v[0, 16 * v + 8:16 * v + 16, :] * cf + e_v[1, 16 * v + 8:16 * v + 16, :] * sf
                mf_v[k1, 8 * v:8 * v + 8, :] = pk2(lo, hi)
            ci = jnp.broadcast_to(cs_v[2, k1:k1 + 1, :], (8, 128)); si = jnp.broadcast_to(cs_v[3, k1:k1 + 1, :], (8, 128))
            nn = jnp.concatenate([e_v[2, 8 * r:8 * r + 8, :] * ci + e_v[3, 8 * r:8 * r + 8, :] * si for r in range(16)], axis=0).T
            for v in range(8):
                mi_v[k1, 8 * v:8 * v + 8, :] = pk2(nn[16 * v:16 * v + 8], nn[16 * v + 8:16 * v + 16])

        def pre(u, kp, p):
            for g in range(8):
                v = [(PR[p, a * 8 + kp, 8 * g:8 * g + 8, :], PI[p, a * 8 + kp, 8 * g:8 * g + 8, :]) for a in range(4)]
                ts = _radix4(v, -1)
                for kk in range(4):
                    TS[u % 2, kk, 8 * g:8 * g + 8, :] = pk2(ts[kk][0], ts[kk][1])

        def fwd(u, kp, p):
            return [jnp.dot(tb(mf_v[kp + 8 * kk]), tb(TS[u % 2, kk]), preferred_element_type=f32) for kk in range(4)]

        def mid(u, kp, p, xs):
            for g in range(8):
                for kk in range(4):
                    k1 = kp + 8 * kk
                    x = xs[kk]
                    xr, xi = x[16 * g:16 * g + 8], x[16 * g + 8:16 * g + 16]
                    ww = WW[p, pl.ds(k1 + 33 * 8 * g, 8, stride=33), :]
                    wr = upk(ww, 0); wi = upk(ww, 1)
                    YS[u % 2, kk, 8 * g:8 * g + 8, :] = pk2(xr * wr - xi * wi, xr * wi + xi * wr)
            return [jnp.dot(tb(mi_v[kp + 8 * kk]), tb(YS[u % 2, kk]), preferred_element_type=f32) for kk in range(4)]

        def post(kp, p, outs):
            for g in range(8):
                v = [(o[16 * g:16 * g + 8], o[16 * g + 8:16 * g + 16]) for o in outs]
                r = _radix4(v, +1)
                for a in range(4):
                    PR[p, a * 8 + kp, 8 * g:8 * g + 8, :] = r[a][0]
                    PI[p, a * 8 + kp, 8 * g:8 * g + 8, :] = r[a][1]

        def inv_fft_half(a, p, j, par):
            xs = []
            rr = pl.ds(16 * j + par, 8, stride=2)
            for kp in range(8):
                v = (PR[p, a * 8 + kp, rr, :], PI[p, a * 8 + kp, rr, :])
                xs.append(_cmul_const(v, 2 * np.pi * a * kp / 32))
            return _fft(xs, +1)

        def inv_unit_p(u, p):
            a, j = fft_units[u]
            ze = inv_fft_half(a, p, j, 0)
            zo = inv_fft_half(a, p, j, 1)
            for b in range(8):
                r = slice(8 * b, 8 * b + 8)
                (er, ei), (orr, oi) = ze[b], zo[b]
                if p == 2:
                    ZS[u % 3, r, 0:128] = pk2(jnp.where(lane8 <= 64, er, pltpu.roll(ei, 64, 1)),
                                              jnp.where(lane8 <= 64, orr, pltpu.roll(oi, 64, 1)))
                elif p == 0:
                    ZS[u % 3, r, 128:256] = pk2(er, orr)
                    ZS[u % 3, r, 256:384] = pk2(ei, oi)
                else:
                    ZS[u % 3, r, 384:512] = pk2(er, orr)
                    ZS[u % 3, r, 512:640] = pk2(ei, oi)

        nt_dims = (((1,), (1,)), ((), ()))

        def dinv_dot(u, n):
            if n == 0:
                return lax.dot_general(tb(ZS[u % 3, :, 128:384]), tb(rd_v[0]), nt_dims, preferred_element_type=f32)
            if n == 1:
                return lax.dot_general(tb(ZS[u % 3, :, 384:640]), tb(rd_v[1]), nt_dims, preferred_element_type=f32)
            return lax.dot_general(tb(ZS[u % 3, :, 0:128]), tb(rd_v[2, 0:64, 0:128]), nt_dims, preferred_element_type=f32)

        def r5_inv(u, qs, bs):
            a, j = fft_units[u]
            q1, q2, q0 = qs
            for b in bs:
                r = slice(16 * b, 16 * b + 16)
                ys = _radix5_inv(q0[r], q1[r, 0:128], q1[r, 128:256], q2[r, 0:128], q2[r, 128:256])
                for t in range(5):
                    Y[0, pl.ds(rows_of(a, b) + 16 * j, 16), 128 * t:128 * t + 128] = ys[t].astype(bf)

        a_out = pltpu.make_async_copy(Y.at[0, pl.ds(128, S_ - 128), :], out_h.at[pl.ds(128, S_ - 128), pl.ds(0, 640)], osem.at[1])
        fft_units = [(a, j) for a in range(4) for j in range(4)]
        a_of = lambda u_: u_ // 4

        def mxu_stage(p, extra):
            st = {}
            for t in range(8 + LA + 1):
                if t < 8: st[t] = ('f', fwd(t, p, pre(t, p)))
                u = t - LA
                if 0 <= u < 8: st[u] = ('m', mid(u, p, st[u][1]))
                u = t - LA - 1
                if 0 <= u < 8: post(u, p, st.pop(u)[1])
                if t < 8: extra(t)

        cp_rd.wait()
        cp_xa[0].wait()
        for c_ in (cp_xa[1], *cp_e, cp_xa[2], cp_xa[3], *cp_wg[0], *cp_wg[1], cp_w, cp_xb[0], cp_wo, cp_xb[1]): c_.start()
        wjobs = [(c, p_) for c in range(16) for p_ in range(3)]

        def wt_job(i, half):
            base = 0 if half == 0 else 1280
            wT[640 * half + 128 * i:640 * half + 128 * i + 128, :] = tb(wqkv_v[:, base + 128 * i:base + 128 * i + 128]).T
        bsplit = [(0, 1, 2), (3, 4, 5), (6, 7)]
        r5_fwd(0, range(8))
        r5_fwd(1, range(8))
        dres = {}
        for q in range(48 + LQ):
            if q < 48:
                u, n = q // 3, q % 3
                dres[q] = dfwd_dot(u, n)
            qq = q - LQ
            if qq < 0: continue
            u, n = qq // 3, qq % 3
            if n == 0:
                if u + 2 < 16 and fft_units[u + 2][1] == 0:
                    cp_xa[fft_units[u + 2][0]].wait()
                if qq == 3 * (MB0 // 3):
                    for c_ in cp_e: c_.wait()
                if u == WU0:
                    for c_ in cp_wg[0]: c_.wait()
            if ORD == 0:
                fwd_fft_unit(a_of(u), n, u % 4, dres.pop(qq))
            if u + 2 < 16: r5_fwd(u + 2, bsplit[n])
            if 0 <= u - WU0 < NWU:
                k_ = (u - WU0) * 3 + n
                for jb in wjobs[(24 * k_) // (3 * NWU):(24 * (k_ + 1)) // (3 * NWU)]: wprep1(*jb)
            if MB0 <= qq < MB0 + 32: mbuild(qq - MB0)
            if ORD == 1:
                fwd_fft_unit(a_of(u), n, u % 4, dres.pop(qq))
        init_pads()
        for c_ in cp_wg[1]: c_.wait()
        for jb in wjobs[24:48]: wprep1(*jb)
        us = [(kp, p) for kp in range(8) for p in range(3)]
        st = {}
        for t in range(24 + LA + 1):
            if t < 24:
                pre(t, *us[t]); st[t] = fwd(t, *us[t])
            u = t - LA
            if 0 <= u < 24: st[u] = mid(u, *us[u], st[u])
            u = t - LA - 1
            if 0 <= u < 24: post(*us[u], st.pop(u))
        cp_w.wait()
        cp_xb[0].wait()
        x0 = tb(xb[0:64, :])
        proj_k(0, x0)
        for p in range(3): inv_unit_p(0, p)
        for p in range(3): inv_unit_p(1, p)
        qres = {}
        for u in range(16 + LI):
            for n in range(3):
                if u < 16: qres[(u, n)] = dinv_dot(u, n)
                if u + 2 < 16: inv_unit_p(u + 2, n)
                ui = u - LI
                if ui >= 0: r5_inv(ui, [qres[(ui, 0)], qres[(ui, 1)], qres[(ui, 2)]], bsplit[n])
                if n == 2 and 1 <= u < 11: wt_job((u - 1) // 2, (u - 1) % 2)
            if u == PQ: proj_qv(0, x0, 0)
        a_out.start()
        cp_wo.wait()
        cp_xb[1].wait()

        def body(b, carry):
            slot = b % 2
            bn = jnp.minimum(b + 1, NB - 1)
            bp = jnp.maximum(b - 1, 0)

            dots = {}; sts = {}; outs = {}
            for t in range(NH + LAG):
                if t < NH: dots[t] = qk_dot(b, t, slot)
                if t == TF: fin_o()
                if t == TO: outproj(bp)
                if 0 <= t - LAG1 < NH: sts[t - LAG1] = max_stage(dots.pop(t - LAG1))
                if t == NH + TK:
                    xn = tb(xb[pl.ds(pl.multiple_of(bn * 64, 64), 64), :])
                    proj_k(bn, xn)
                if TQ >= 0 and t == NH + TQ:
                    proj_qv(bn, xn, 1 - slot)
                if 0 <= t - LAG < NH:
                    h = t - LAG
                    outs[h] = exp_pv(b, h, sts.pop(h))
                    if h % 2 == 1:
                        A = outs.pop(h - 1); B = outs.pop(h)
                        p = h // 2
                        OT[40 * p:40 * p + 40, :] = jnp.concatenate([A[0:16], jnp.where(sub8 < 4, A[16:24], B[0:8]), B[8:24]], axis=0)
            if TQ < 0: proj_qv(bn, xn, 1 - slot)
            out_copy(bp, jnp.minimum(b, 1)).start()
            return carry
        lax.fori_loop(0, NB, body, 0, unroll=UNR)
        fin_o()
        outproj(NB - 1)
        out_copy(NB - 1, 1).start()
        a_out.wait()
        for i in range(NB + 1):
            out_copy(0, 1).wait()
    return kernel


def run(A_x, A_w_r, A_w_i, B_x, B_wqkv, B_wo, **kw):
    kernel = make_kernel(**kw)
    hbm = pl.BlockSpec(memory_space=pltpu.HBM)
    V = pltpu.VMEM
    wrT, wiT = A_w_r.T, A_w_i.T
    out = pl.pallas_call(
        kernel,
        out_shape=jax.ShapeDtypeStruct((S_, 2 * D), bf),
        in_specs=[hbm] * 9, out_specs=hbm,
        scratch_shapes=[
            V((4, 8, 32, D), jnp.uint32), V((16, 160, 128), jnp.uint32), V((16, 160, 128), jnp.uint32),
            V((3, 128, 256), jnp.uint32), V((R, 64, 128), jnp.uint32), V((R, 64, 128), jnp.uint32),
            V((4, 128, 128), f32), V((4, R, 128), f32), V((1, S_), bf), V((1, S_), bf),
            V((3, 32, 64, 128), f32), V((3, 32, 64, 128), f32),
            V((3, 2112, 128), jnp.uint32),
            V((2, S_, D), bf), V((2, 4, 64, 128), jnp.uint32), V((2, 4, 64, 128), jnp.uint32), V((3, 64, D), jnp.uint32), V((3, 64, D), jnp.uint32),
            V((S_ // 2, D), jnp.uint32), V((D // 2, 3 * D), jnp.uint32), V((D // 2, D), jnp.uint32), V((2 * D, D), bf),
            V((NB + 2, 128, 1024), bf), V((NB + 2, 1024, 128), bf),
            V((2, D, 128), f32), V((D, 128), f32), V((128, D), bf),
            pltpu.SemaphoreType.DMA((13,)), pltpu.SemaphoreType.DMA((2,)),
        ],
        compiler_params=pltpu.CompilerParams(vmem_limit_bytes=110 * 2**20),
        name='fused',
    )(A_x.reshape(8, 4, 64, D), wrT, wiT, B_x.reshape(S_, D), B_wqkv, B_wo,
      jnp.asarray(RD_U32), jnp.asarray(E_NP), jnp.asarray(CS_NP))
    return out.reshape(1, S_, 2 * D)


@jax.jit
def pallas_concat_heads__spectral_gfnet__sliding_block__prompt_kernel(
    A_x: jax.Array,
    A_w_r: jax.Array,
    A_w_i: jax.Array,
    B_x: jax.Array,
    B_wqkv: jax.Array,
    B_wo: jax.Array,
):
    return run(A_x, A_w_r, A_w_i, B_x, B_wqkv, B_wo, UNR=4, LAG=10, WU0=12, NWU=4, MB0=6)
```

```python
import numpy as np
import jax
import jax.numpy as jnp
from jax import lax
import jax.experimental.pallas as pl
import jax.experimental.pallas.tpu as pltpu

bf = jnp.bfloat16
f32 = jnp.float32
S_ = 2048
D = 640
NB = 16
NH = 32
R = 32
QSCALE = float((20 ** -0.5) * np.log2(np.e))
NEG = -1e30


def _consts():
    n2 = np.arange(128)[:, None].astype(np.float64)

    m_ = np.arange(32)

    def gmat(r1, r2):
        l = np.concatenate([r1 + 10 * m_, r1 + 5 + 10 * m_, r2 + 10 * m_, r2 + 5 + 10 * m_]).astype(np.float64)[None, :]
        c = np.cos(2 * np.pi * n2 * l / D); s = np.sin(2 * np.pi * n2 * l / D)
        sg = np.concatenate([np.ones(64), -np.ones(64)])[None, :]
        return np.block([[c, -s], [sg * s, sg * c]])
    g = np.zeros((3, 256, 256))
    g[0] = gmat(1, 4)
    g[1] = gmat(2, 3)
    l0 = np.concatenate([10 * m_, 5 + 10 * m_]).astype(np.float64)[None, :]
    g0 = np.concatenate([np.cos(2 * np.pi * n2 * l0 / D), -np.sin(2 * np.pi * n2 * l0 / D)], axis=1)
    g0[:, 64] = np.cos(np.pi * n2[:, 0])
    g[2, :128, :128] = g0
    perm_out = np.array([64 * ((r % 16) // 8) + 8 * (r // 16) + (r % 8) for r in range(128)])
    perm_in = perm_out
    pre = np.array([16 * (r // 16) + 2 * (r % 8) + ((r % 16) // 8) for r in range(128)])
    k2 = np.arange(64)[:, None]; s2 = np.arange(64)[None, :]
    F = np.exp(-2j * np.pi * ((s2 * k2) % 64) / 64)
    e1 = np.block([[F.real, -F.imag], [F.imag, F.real]])
    e2 = np.block([[-F.imag, -F.real], [F.real, -F.imag]])
    rows_f = perm_out[pre]
    cols_i = perm_out[pre]
    E = np.stack([e1[rows_f][:, perm_in], e2[rows_f][:, perm_in], e1[perm_in][:, cols_i], e2[perm_in][:, cols_i]])
    s2f = perm_in % 64; s2i = cols_i % 64
    k1 = np.arange(R)[:, None]
    CS = np.stack([np.cos(2 * np.pi * ((k1 * s2f[None, :]) % S_) / S_), -np.sin(2 * np.pi * ((k1 * s2f[None, :]) % S_) / S_),
                   np.cos(2 * np.pi * ((k1 * s2i[None, :]) % S_) / S_), -np.sin(2 * np.pi * ((k1 * s2i[None, :]) % S_) / S_)])
    b16 = jnp.bfloat16
    return g.astype(np.float32).astype(b16), E.astype(np.float32), CS.astype(np.float32)


RD_NP, E_NP, CS_NP = _consts()
SIG = float(2.0 / (S_ * D))
C1, C2 = float(np.cos(2 * np.pi / 5)), float(np.cos(4 * np.pi / 5))
S1, S2 = float(np.sin(2 * np.pi / 5)), float(np.sin(4 * np.pi / 5))


def _radix5_fwd(x):
    t1, t2 = x[1] + x[4], x[2] + x[3]
    t3, t4 = x[1] - x[4], x[2] - x[3]
    a0 = x[0] + t1 + t2
    a1 = x[0] + C1 * t1 + C2 * t2
    a2 = x[0] + C2 * t1 + C1 * t2
    b1 = -(S1 * t3 + S2 * t4)
    b2 = S1 * t4 - S2 * t3
    return [a0, a1, b1, a2, b2]


def _radix5_inv(q0, q1r, q1i, q2r, q2i):
    q0s = SIG * q0
    t1 = q0s + (SIG * C1) * q1r + (SIG * C2) * q2r
    t2 = q0s + (SIG * C2) * q1r + (SIG * C1) * q2r
    u1 = (SIG * S1) * q1i + (SIG * S2) * q2i
    u2 = (SIG * S2) * q1i - (SIG * S1) * q2i
    return [SIG * (q0 + q1r + q2r), t1 - u1, t2 - u2, t2 + u2, t1 + u1]


def _pack_rows_u32(m):
    u = m.view(np.uint16).astype(np.uint32)
    return (u[..., 0::2, :] | (u[..., 1::2, :] << 16)).astype(np.uint32)


RD_U32 = _pack_rows_u32(RD_NP)


def _cmul_const(v, ang):
    re, im = v
    c, s = float(np.cos(ang)), float(np.sin(ang))
    eps = 1e-12
    if abs(s) < eps:
        return (re, im) if c > 0 else (-re, -im)
    if abs(c) < eps:
        return (-im, re) if s > 0 else (im, -re)
    if abs(abs(c) - abs(s)) < eps:
        h = abs(c)
        if c > 0 and s > 0: return ((re - im) * h, (re + im) * h)
        if c > 0 and s < 0: return ((re + im) * h, (im - re) * h)
        if c < 0 and s > 0: return ((re + im) * (-h), (re - im) * h)
        return ((im - re) * h, (re + im) * (-h))
    return (re * c - im * s, re * s + im * c)


def _fft(xs, sign):
    n = len(xs)
    if n == 1:
        return xs
    ev = _fft(xs[0::2], sign); od = _fft(xs[1::2], sign)
    out = [None] * n
    for k in range(n // 2):
        er, ei = ev[k]; orr, oi = od[k]
        if 4 * k == n:
            if sign < 0:
                out[k] = (er + oi, ei - orr); out[k + n // 2] = (er - oi, ei + orr)
            else:
                out[k] = (er - oi, ei + orr); out[k + n // 2] = (er + oi, ei - orr)
        else:
            tr, ti = _cmul_const((orr, oi), sign * 2 * np.pi * k / n)
            out[k] = (er + tr, ei + ti); out[k + n // 2] = (er - tr, ei - ti)
    return out


def _radix4(v, sign):
    (ar, ai), (br, bi), (cr, ci), (dr, di) = v
    s0r, s0i = ar + cr, ai + ci
    s1r, s1i = ar - cr, ai - ci
    s2r, s2i = br + dr, bi + di
    s3r, s3i = br - dr, bi - di
    o0 = (s0r + s2r, s0i + s2i)
    o2 = (s0r - s2r, s0i - s2i)
    if sign < 0:
        o1 = (s1r + s3i, s1i - s3r); o3 = (s1r - s3i, s1i + s3r)
    else:
        o1 = (s1r - s3i, s1i + s3r); o3 = (s1r + s3i, s1i - s3r)
    return [o0, o1, o2, o3]


def make_kernel(LAG=8, LAG1=2, TK=0, LA=2, WU0=11, NWU=5, MB0=8, EW=2, MORD=1, PK=0, PQ=13, UNR=1, LQ=1, ORD=1, LI=1, TO=2, TF=0, TQ=-1):
    def kernel(ax_h, wr_h, wi_h, bx_h, wqkv_h, wo_h, rd_h, e_h, cs_h, out_h,
               xa, wr_v, wi_v, rd_v, mf_v, mi_v, e_v, cs_v, PR, PI, WW, Y, TS, YS, ZF, XL, WU,
               xb, wqkv_v, wo_v, wT, KP, VT, QT, OT, OS, sems, osem):
        cp = lambda s_, d_, i: pltpu.make_async_copy(s_, d_, sems.at[i])
        cp_rd = cp(rd_h, rd_v, 0)
        cp_xa = [cp(ax_h.at[:, i], xa.at[i], 1 + i) for i in range(4)]
        cp_wg = [[cp(h_.at[:, pl.ds(1024 * g_, 1024)], v_.at[g_], 5 + g_) for (h_, v_) in ((wr_h, wr_v), (wi_h, wi_v))]
                 for g_ in range(2)]
        cp_e = [cp(e_h, e_v, 7), cp(cs_h, cs_v, 7)]
        cp_w = cp(wqkv_h, wqkv_v, 9)
        cp_xb = [cp(bx_h.at[pl.ds(0, 256), :], xb.at[pl.ds(0, 256), :], 9),
                 cp(bx_h.at[pl.ds(256, 1792), :], xb.at[pl.ds(256, 1792), :], 10)]
        cp_wo = cp(wo_h, wo_v, 10)
        for c_ in (cp_rd, cp_xa[0], cp_xa[1], *cp_e, cp_xa[2], cp_xa[3], *cp_wg[0], *cp_wg[1], cp_w, cp_xb[0], cp_wo, cp_xb[1]): c_.start()

        tb = lambda v: pltpu.bitcast(v, bf)
        u32 = jnp.uint32
        HI = jnp.uint32(0xffff0000)

        def pk2(a_, b_):
            ua = pltpu.bitcast(a_, u32) + jnp.uint32(0x8000)
            ub = pltpu.bitcast(b_, u32) + jnp.uint32(0x8000)
            return (ua >> 16) | (ub & HI)

        def upk(w_, i_):
            return pltpu.bitcast(w_ << 16, f32) if i_ == 0 else pltpu.bitcast(w_ & HI, f32)
        sub8 = lax.broadcasted_iota(jnp.int32, (8, 128), 0)
        col8 = lax.broadcasted_iota(jnp.int32, (8, 128), 1)
        lane = lax.broadcasted_iota(jnp.int32, (128, 128), 1)
        lane16 = lax.broadcasted_iota(jnp.int32, (16, 128), 1)

        def init_pads():
            lane_k = lax.broadcasted_iota(jnp.int32, (128, 1024), 1)
            kpad = jnp.where((lane_k % 128) == 127, NEG, 0.0).astype(bf)
            KP[0] = kpad; KP[1] = kpad
            VT[0] = jnp.zeros((1024, 128), bf); VT[1] = jnp.zeros((1024, 128), bf)
            OT[...] = jnp.zeros(OT.shape, f32)

        def proj_k(b, xblk):
            kf = jnp.dot(xblk, wqkv_v[:, 640:1280], preferred_element_type=f32)
            for g in range(8):
                off = 80 * g; t = off // 128; sh = off % 128
                s0 = kf[:, 128 * t:128 * t + 128]
                if sh: s0 = pltpu.roll(s0, 128 - sh, 1)
                if sh + 80 > 128:
                    s1 = pltpu.roll(kf[:, 128 * (t + 1):128 * (t + 2)], 128 - sh, 1)
                    tile = jnp.where(lane < 128 - sh, s0, jnp.where(lane < 80, s1, 0.0))
                else:
                    tile = jnp.where(lane < 80, s0, 0.0)
                KP[b + 2, :, 128 * g:128 * g + 128] = tile.astype(bf)

        def proj_qv(b, xblk, slot):
            nt = lambda lo, n: lax.dot_general(wT[lo:lo + n, :], xblk, (((1,), (1,)), ((), ())), preferred_element_type=f32)
            QT[slot, 0:320, :] = nt(0, 320) * QSCALE
            QT[slot, 320:640, :] = nt(320, 320) * QSCALE
            vv = jnp.concatenate([nt(640, 320), nt(960, 320)], axis=0)
            cA = jnp.where(sub8 == 4, 1.0, 0.0).astype(f32)
            cB = jnp.where(sub8 == 0, 1.0, 0.0).astype(f32)
            z8 = jnp.zeros((8, 128), f32)
            for p in range(16):
                v = [vv[40 * p + 8 * i: 40 * p + 8 * i + 8] for i in range(5)]
                blk = jnp.concatenate([v[0], v[1], jnp.where(sub8 < 4, v[2], cA), z8,
                                       jnp.where(sub8 >= 4, v[2], cB), v[3], v[4], z8], axis=0)
                VT[b + 2, 64 * p:64 * p + 64, :] = blk.astype(bf)

        def build_w(h, slot):
            g, i = h // 4, h % 4
            a = (20 * i) // 16
            q = QT[slot, g * 80 + 16 * a: g * 80 + 16 * a + 32, :]
            r = lax.broadcasted_iota(jnp.int32, (32, 128), 0) + 16 * a
            qm = jnp.where((r >= 20 * i) & (r < 20 * i + 20), q, 0.0)
            parts = []
            if a > 0: parts.append(jnp.zeros((16 * a, 128), f32))
            parts.append(qm)
            parts.append(jnp.zeros((120 - 16 * a - 32, 128), f32))
            parts.append(jnp.where(sub8 == 7, 1.0, 0.0).astype(f32))
            return jnp.concatenate(parts, axis=0).astype(bf)

        lane64 = lax.broadcasted_iota(jnp.int32, (64, 128), 1)

        def build_wd(h, slot):
            g, i = h // 4, h % 4
            a = (20 * i) // 16
            q = QT[slot, g * 80 + 16 * a: g * 80 + 16 * a + 32, :]
            r = lax.broadcasted_iota(jnp.int32, (32, 128), 0) + 16 * a
            c = lax.broadcasted_iota(jnp.int32, (32, 128), 1)
            qf = jnp.where((r >= 20 * i) & (r < 20 * i + 20) & (c < 64), q, 0.0)
            o_ = (20 * i) % 8
            q2 = QT[slot, g * 80 + 20 * i - o_: g * 80 + 20 * i - o_ + 24, :]
            r2 = lax.broadcasted_iota(jnp.int32, (24, 128), 0)
            c2 = lax.broadcasted_iota(jnp.int32, (24, 128), 1)
            ql = jnp.where((r2 >= o_) & (r2 < o_ + 20) & (c2 >= 64), q2, 0.0)
            parts = []
            if a > 0: parts.append(jnp.zeros((16 * a, 128), f32))
            parts.append(qf)
            if 80 - 16 * a - 32 > 0: parts.append(jnp.zeros((80 - 16 * a - 32, 128), f32))
            parts.append(ql)
            parts.append(jnp.zeros((16, 128), f32))
            parts.append(jnp.where((sub8 == 7) & (col8 < 64), 1.0, 0.0).astype(f32))
            return jnp.concatenate(parts, axis=0).astype(bf)

        lane32 = lax.broadcasted_iota(jnp.int32, (32, 128), 1)

        def build_wd2(h, slot):
            g, i = h // 4, h % 4
            o_ = (20 * i) % 8
            q2 = QT[slot, g * 80 + 20 * i - o_: g * 80 + 20 * i - o_ + 24, :]
            r2 = lax.broadcasted_iota(jnp.int32, (24, 128), 0)
            c2 = lax.broadcasted_iota(jnp.int32, (24, 128), 1)
            rm = (r2 >= o_) & (r2 < o_ + 20)
            parts = [jnp.where(rm & (c2 >= 32 * s_) & (c2 < 32 * s_ + 32), q2, 0.0) for s_ in range(4)]
            parts.append(jnp.zeros((24, 128), f32))
            parts.append(jnp.where((sub8 == 7) & ((col8 // 32) % 2 == 0), 1.0, 0.0).astype(f32))
            return jnp.concatenate(parts, axis=0).astype(bf)

        def qk_dot(b, h, slot):
            g, i = h // 4, h % 4
            w = build_w(h, slot)
            lo, hi = g * 128, (g + 1) * 128
            kt = jnp.concatenate([KP[b + 2, 0:32, lo:hi], KP[b, 96:128, lo:hi], KP[b + 1, :, lo:hi]], axis=0)
            main = jnp.dot(kt, w, preferred_element_type=f32)
            sh = 80 + (20 * i) % 8 - 20 * i
            rl = pltpu.roll(KP[b + 2, 32:96, lo:hi], sh, 1)
            ld = jnp.where((lane64 >= 80) & (lane64 < 104), rl, KP[b, 32:96, lo:hi])
            comb = jnp.dot(ld, build_wd(h, slot), preferred_element_type=f32)
            o_ = (20 * i) % 8
            srcs = [KP[b, 0:32, lo:hi], KP[b + 2, 32:64, lo:hi], KP[b, 64:96, lo:hi], KP[b + 2, 96:128, lo:hi]]
            l2 = None
            for s_ in range(4):
                d_ = 24 * s_ + o_
                shift = (d_ - 20 * i) % 128
                v = pltpu.roll(srcs[s_], shift, 1) if shift else srcs[s_]
                if s_ == 0:
                    l2 = jnp.where(lane32 == 127, srcs[0], v) if shift else v
                else:
                    l2 = jnp.where((lane32 >= d_) & (lane32 < d_ + 20), v, l2)
            diag = jnp.dot(l2, build_wd2(h, slot), preferred_element_type=f32)
            return main, comb, diag

        def max_stage(sd):
            si, cb, dg = sd
            mx = None; scs = []
            for a in range(16):
                tri = sub8 + 8 * a > col8
                d_ = dg[8 * (a % 4):8 * (a % 4) + 8]
                if a < 4: sc = jnp.where(tri, d_, si[8 * a:8 * a + 8])
                elif a < 8: sc = jnp.where((col8 >= 32) & (col8 < 64) & jnp.logical_not(tri), d_, cb[8 * a - 32:8 * a - 24])
                elif a < 12: sc = jnp.where((col8 >= 64) & (col8 < 96) & tri, d_, cb[8 * a - 32:8 * a - 24])
                else: sc = jnp.where(tri, si[8 * a - 64:8 * a - 56], d_)
                scs.append(sc)
                mx = sc if mx is None else jnp.maximum(mx, sc)
            sm = si[64:192]
            for a in range(16):
                mx = jnp.maximum(mx, sm[8 * a:8 * a + 8])
            mx = jnp.max(mx, axis=0, keepdims=True)
            return (jnp.concatenate(scs, axis=0), sm, mx)

        def exp_pv(b, h, st):
            sc, sm, m = st
            row = lax.broadcasted_iota(jnp.int32, (128, 128), 0)
            pc = jnp.exp2(sc - m)
            pm = jnp.exp2(sm - m)
            msk = row > lane
            pu = jnp.where(msk, pc, 0.0)
            pl_ = jnp.where(msk, 0.0, pc)
            pall = jnp.concatenate([pu, pm, pl_], axis=0).astype(bf)
            vt = jnp.concatenate([VT[b + t, 32 * h:32 * h + 32, :] for t in range(3)], axis=1)
            o = jnp.dot(vt, pall, preferred_element_type=f32)
            l = o[20:21, :] if h % 2 == 0 else o[0:1, :]
            r = pltpu.reciprocal(l, approx=False)
            return o[0:24] * r

        def fin_o():
            for kt in range(5):
                OS[:, 128 * kt:128 * kt + 128] = OT[128 * kt:128 * kt + 128, :].T.astype(bf)

        def outproj(bprev):
            y = jnp.dot(OS[...], wo_v[...], preferred_element_type=f32)
            Y[1, pl.ds(pl.multiple_of(bprev * 128, 128), 128), :] = y.astype(bf)

        def out_copy(bb, half):
            return pltpu.make_async_copy(Y.at[half, pl.ds(pl.multiple_of(bb * 128, 128), 128), :],
                                         out_h.at[pl.ds(pl.multiple_of(bb * 128, 128), 128), pl.ds(pl.multiple_of(640 * half, 128), 640)], osem.at[0])

        def rows_of(a, b):
            return 64 * (a + 4 * b)

        xau = xa

        def r5_fwd(u, bs):
            a, j = fft_units[u]
            for b in bs:
                xs = [xa[a, b, 16 * j:16 * j + 16, 128 * t:128 * t + 128].astype(f32) for t in range(5)]
                o = _radix5_fwd(xs)
                for t in range(5):
                    XL[u % 3, 16 * b:16 * b + 16, 128 * t:128 * t + 128] = o[t].astype(bf)

        def dfwd_dot(u, n):
            if n == 0:
                r_ = jnp.dot(XL[u % 3, :, 128:384], tb(rd_v[0]), preferred_element_type=f32)
                return (r_[:, 0:128], r_[:, 128:256])
            if n == 1:
                r_ = jnp.dot(XL[u % 3, :, 384:640], tb(rd_v[1]), preferred_element_type=f32)
                return (r_[:, 0:128], r_[:, 128:256])
            return jnp.dot(XL[u % 3, :, 0:128], tb(rd_v[2, 0:64, 0:128]), preferred_element_type=f32)

        lane8 = col8

        def fwd_fft_unit(a, p, j, t):
          for hh in range(2):
            xs = []
            for b in range(8):
                r = slice(16 * b + 8 * hh, 16 * b + 8 * hh + 8)
                if p < 2:
                    re = t[0][r]; im = t[1][r]
                else:
                    m = t[r]
                    re = jnp.where(lane8 <= 64, m, 0.0)
                    im = jnp.where((lane8 >= 1) & (lane8 < 64), pltpu.roll(m, 64, 1), 0.0)
                xs.append((re, im))
            ys = _fft(xs, -1)
            for kp in range(8):
                y = _cmul_const(ys[kp], -2 * np.pi * a * kp / 32)
                rr = slice(16 * j + 8 * hh, 16 * j + 8 * hh + 8)
                PR[p, a * 8 + kp, rr, :] = y[0]
                PI[p, a * 8 + kp, rr, :] = y[1]

        def wretile(c):
            cs = slice(128 * (c % 8), 128 * (c % 8) + 128)
            WU[c, 0] = pltpu.bitcast(wr_v[c // 8, 0:320, cs], u32)
            WU[c, 1] = pltpu.bitcast(wi_v[c // 8, 0:320, cs], u32)

        def wprep1(c, p):
            def rows(rho):
                sl = pl.ds(rho // 2, 32, stride=5)
                a_ = upk(WU[c, 0, sl, :], rho % 2); b_ = upk(WU[c, 1, sl, :], rho % 2)
                if rho == 0:
                    r32 = lax.broadcasted_iota(jnp.int32, (32, 128), 0)
                    a_ = jnp.where(r32 == 0, 0.5 * a_, a_); b_ = jnp.where(r32 == 0, 0.5 * b_, b_)
                return (pltpu.bitcast(a_, u32) >> 16) | pltpu.bitcast(b_, u32)
            if p < 2:
                r1, r2 = (1, 4) if p == 0 else (2, 3)
                w = jnp.concatenate([rows(r1), rows(r1 + 5), rows(r2), rows(r2 + 5)], axis=0)
            else:
                cs = slice(128 * (c % 8), 128 * (c % 8) + 128)
                a_ = jnp.where(sub8 == 0, 0.5 * jnp.broadcast_to(wr_v[c // 8, 320:321, cs].astype(f32), (8, 128)), 0.0)
                b_ = jnp.where(sub8 == 0, 0.5 * jnp.broadcast_to(wi_v[c // 8, 320:321, cs].astype(f32), (8, 128)), 0.0)
                nyq = (pltpu.bitcast(a_, u32) >> 16) | pltpu.bitcast(b_, u32)
                w = jnp.concatenate([rows(0), rows(5), nyq, jnp.zeros((56, 128), u32)], axis=0)
            w = w.T
            for q in range(4):
                WW[p, pl.ds(33 * (4 * c + q), 32), :] = w[32 * q:32 * q + 32]

        def mbuild(k1):
            cf = jnp.broadcast_to(cs_v[0, k1:k1 + 1, :], (8, 128)); sf = jnp.broadcast_to(cs_v[1, k1:k1 + 1, :], (8, 128))
            for v in range(8):
                lo = e_v[0, 16 * v:16 * v + 8, :] * cf + e_v[1, 16 * v:16 * v + 8, :] * sf
                hi = e_v[0, 16 * v + 8:16 * v + 16, :] * cf + e_v[1, 16 * v + 8:16 * v + 16, :] * sf
                mf_v[k1, 8 * v:8 * v + 8, :] = pk2(lo, hi)
            ci = jnp.broadcast_to(cs_v[2, k1:k1 + 1, :], (8, 128)); si = jnp.broadcast_to(cs_v[3, k1:k1 + 1, :], (8, 128))
            nn = jnp.concatenate([e_v[2, 8 * r:8 * r + 8, :] * ci + e_v[3, 8 * r:8 * r + 8, :] * si for r in range(16)], axis=0).T
            for v in range(8):
                mi_v[k1, 8 * v:8 * v + 8, :] = pk2(nn[16 * v:16 * v + 8], nn[16 * v + 8:16 * v + 16])

        def pre(u, kp, p):
            for g in range(8):
                v = [(PR[p, a * 8 + kp, 8 * g:8 * g + 8, :], PI[p, a * 8 + kp, 8 * g:8 * g + 8, :]) for a in range(4)]
                ts = _radix4(v, -1)
                for kk in range(4):
                    TS[u % 2, kk, 16 * g:16 * g + 16, :] = jnp.concatenate([ts[kk][0], ts[kk][1]], axis=0).astype(bf)

        def fwd(u, kp, p):
            return [jnp.dot(tb(mf_v[kp + 8 * kk]), TS[u % 2, kk], preferred_element_type=f32) for kk in range(4)]

        def mid(u, kp, p, xs):
            for g in range(8):
                for kk in range(4):
                    k1 = kp + 8 * kk
                    x = xs[kk]
                    xr, xi = x[16 * g:16 * g + 8], x[16 * g + 8:16 * g + 16]
                    ww = WW[p, pl.ds(k1 + 33 * 8 * g, 8, stride=33), :]
                    wr = upk(ww, 0); wi = upk(ww, 1)
                    YS[u % 2, kk, 16 * g:16 * g + 16, :] = jnp.concatenate([xr * wr - xi * wi, xr * wi + xi * wr], axis=0).astype(bf)

        def inv(u, kp, p):
            return [jnp.dot(tb(mi_v[kp + 8 * kk]), YS[u % 2, kk], preferred_element_type=f32) for kk in range(4)]

        def post(kp, p, outs):
            for g in range(8):
                v = [(o[16 * g:16 * g + 8], o[16 * g + 8:16 * g + 16]) for o in outs]
                r = _radix4(v, +1)
                for a in range(4):
                    PR[p, a * 8 + kp, 8 * g:8 * g + 8, :] = r[a][0]
                    PI[p, a * 8 + kp, 8 * g:8 * g + 8, :] = r[a][1]

        def inv_unit_p(u, p):
            a, j = fft_units[u]
            for hh in range(2):
                rr = slice(16 * j + 8 * hh, 16 * j + 8 * hh + 8)
                xs = []
                for kp in range(8):
                    v = (PR[p, a * 8 + kp, rr, :], PI[p, a * 8 + kp, rr, :])
                    xs.append(_cmul_const(v, 2 * np.pi * a * kp / 32))
                zs = _fft(xs, +1)
                for b in range(8):
                    r = slice(16 * b + 8 * hh, 16 * b + 8 * hh + 8)
                    zr, zi = zs[b]
                    if p == 2:
                        ZF[u % 3, r, 0:128] = jnp.where(lane8 <= 64, zr, pltpu.roll(zi, 64, 1))
                    elif p == 0:
                        ZF[u % 3, r, 128:256] = zr
                        ZF[u % 3, r, 256:384] = zi
                    else:
                        ZF[u % 3, r, 384:512] = zr
                        ZF[u % 3, r, 512:640] = zi

        nt_dims = (((1,), (1,)), ((), ()))

        def dinv_dot(u, n):
            if n == 0:
                return lax.dot_general(ZF[u % 3, :, 128:384].astype(bf), tb(rd_v[0]), nt_dims, preferred_element_type=f32)
            if n == 1:
                return lax.dot_general(ZF[u % 3, :, 384:640].astype(bf), tb(rd_v[1]), nt_dims, preferred_element_type=f32)
            return lax.dot_general(ZF[u % 3, :, 0:128].astype(bf), tb(rd_v[2, 0:64, 0:128]), nt_dims, preferred_element_type=f32)

        def r5_inv(u, qs, bs):
            a, j = fft_units[u]
            q1, q2, q0 = qs
            for b in bs:
                r = slice(16 * b, 16 * b + 16)
                ys = _radix5_inv(q0[r], q1[r, 0:128], q1[r, 128:256], q2[r, 0:128], q2[r, 128:256])
                for t in range(5):
                    Y[0, pl.ds(rows_of(a, b) + 16 * j, 16), 128 * t:128 * t + 128] = ys[t].astype(bf)

        a_out = pltpu.make_async_copy(Y.at[0, pl.ds(128, S_ - 128), :], out_h.at[pl.ds(128, S_ - 128), pl.ds(0, 640)], osem.at[1])
        fft_units = [(a, j) for a in range(4) for j in range(4)]
        a_of = lambda u_: u_ // 4

        def mxu_stage(p, extra):
            st = {}
            for t in range(8 + LA + 1):
                if t < 8: st[t] = ('f', fwd(t, p, pre(t, p)))
                u = t - LA
                if 0 <= u < 8: st[u] = ('m', mid(u, p, st[u][1]))
                u = t - LA - 1
                if 0 <= u < 8: post(u, p, st.pop(u)[1])
                if t < 8: extra(t)

        init_pads()
        cp_rd.wait()
        cp_xa[0].wait()
        wjobs = [(c, p_) for c in range(16) for p_ in range(3)]

        def wt_job(i, half):
            base = 0 if half == 0 else 1280
            wT[640 * half + 128 * i:640 * half + 128 * i + 128, :] = wqkv_v[:, base + 128 * i:base + 128 * i + 128].T
        bsplit = [(0, 1, 2), (3, 4, 5), (6, 7)]
        r5_fwd(0, range(8))
        r5_fwd(1, range(8))
        dres = {}
        for q in range(48 + LQ):
            qq = q - LQ
            if qq >= 0 and qq % 3 == 0:
                u = qq // 3
                if u + 2 < 16 and fft_units[u + 2][1] == 0:
                    cp_xa[fft_units[u + 2][0]].wait()
                if u == EW:
                    for c_ in cp_e: c_.wait()
                if u == WU0:
                    for c_ in cp_wg[0]: c_.wait()
            if q < 48:
                dres[q] = dfwd_dot(q // 3, q % 3)
            if qq < 0: continue
            u, n = qq // 3, qq % 3
            if ORD == 0:
                fwd_fft_unit(a_of(u), n, u % 4, dres.pop(qq))
            if u + 2 < 16: r5_fwd(u + 2, bsplit[n])
            if 0 <= u - WU0 < NWU:
                k_ = (u - WU0) * 3 + n
                if k_ == 0:
                    for c_i in range(8): wretile(c_i)
                for jb in wjobs[(24 * k_) // (3 * NWU):(24 * (k_ + 1)) // (3 * NWU)]: wprep1(*jb)
            if MB0 <= qq < MB0 + 32: mbuild(qq - MB0)
            if ORD == 1:
                fwd_fft_unit(a_of(u), n, u % 4, dres.pop(qq))
        for c_ in cp_wg[1]: c_.wait()
        for c_i in range(8, 16): wretile(c_i)
        for jb in wjobs[24:48]: wprep1(*jb)
        us = [(kp, p) for kp in range(8) for p in range(3)]
        st = {}
        if MORD == 0:
            for t in range(24 + LA + 1):
                if t < 24:
                    pre(t, *us[t]); st[t] = fwd(t, *us[t])
                u = t - LA
                if 0 <= u < 24:
                    mid(u, *us[u], st[u]); st[u] = inv(u, *us[u])
                u = t - LA - 1
                if 0 <= u < 24: post(*us[u], st.pop(u))
        else:
            xr_ = {}; or_ = {}
            pre(0, *us[0])
            for t in range(24 + 2):
                if t < 24: xr_[t] = fwd(t, *us[t])
                if MORD == 1:
                    if t >= 2: post(*us[t - 2], or_.pop(t - 2))
                    if t + 1 < 24: pre(t + 1, *us[t + 1])
                else:
                    if t + 1 < 24: pre(t + 1, *us[t + 1])
                    if t >= 2: post(*us[t - 2], or_.pop(t - 2))
                if 1 <= t <= 24: or_[t - 1] = inv(t - 1, *us[t - 1])
                if t < 24: mid(t, *us[t], xr_.pop(t))
        cp_w.wait()
        cp_xb[0].wait()
        x0 = xb[0:128, :]
        proj_k(0, x0)
        for p in range(3): inv_unit_p(0, p)
        for p in range(3): inv_unit_p(1, p)
        qres = {}
        for u in range(16 + LI):
            for n in range(3):
                if u < 16: qres[(u, n)] = dinv_dot(u, n)
                if u + 2 < 16: inv_unit_p(u + 2, n)
                ui = u - LI
                if ui >= 0: r5_inv(ui, [qres[(ui, 0)], qres[(ui, 1)], qres[(ui, 2)]], bsplit[n])
                if n == 2 and 1 <= u < 11: wt_job((u - 1) // 2, (u - 1) % 2)
            if u == PQ: proj_qv(0, x0, 0)
        a_out.start()
        cp_wo.wait()
        cp_xb[1].wait()

        def step(b, last):
            slot = b % 2
            bp = b - 1 if last else jnp.maximum(b - 1, 0)
            dots = {}; sts = {}; outs = {}
            if not last:
                bn = b + 1
            for t in range(NH + LAG):
                if t < NH: dots[t] = qk_dot(b, t, slot)
                if t == TF: fin_o()
                if t == TO: outproj(bp)
                if 0 <= t - LAG1 < NH: sts[t - LAG1] = max_stage(dots.pop(t - LAG1))
                if t == NH + TK and not last:
                    xn = xb[pl.ds(pl.multiple_of(bn * 128, 128), 128), :]
                    proj_k(bn, xn)
                if 0 <= t - LAG < NH:
                    h = t - LAG
                    outs[h] = exp_pv(b, h, sts.pop(h))
                    if h % 2 == 1:
                        A = outs.pop(h - 1); B = outs.pop(h)
                        p = h // 2
                        OT[40 * p:40 * p + 40, :] = jnp.concatenate([A[0:16], jnp.where(sub8 < 4, A[16:24], B[0:8]), B[8:24]], axis=0)
            if last:
                out_copy(bp, 1).start()
            else:
                proj_qv(bn, xn, 1 - slot)
                out_copy(bp, jnp.minimum(b, 1)).start()

        def body(b, carry):
            step(b, False)
            return carry
        lax.fori_loop(0, NB - 1, body, 0, unroll=UNR)
        step(NB - 1, True)
        fin_o()
        outproj(NB - 1)
        out_copy(NB - 1, 1).start()
        a_out.wait()
        for i in range(NB + 1):
            out_copy(0, 1).wait()
    return kernel


def run(A_x, A_w_r, A_w_i, B_x, B_wqkv, B_wo, **kw):
    kernel = make_kernel(**kw)
    hbm = pl.BlockSpec(memory_space=pltpu.HBM)
    V = pltpu.VMEM
    wrT, wiT = A_w_r.T, A_w_i.T
    out = pl.pallas_call(
        kernel,
        out_shape=jax.ShapeDtypeStruct((S_, 2 * D), bf),
        in_specs=[hbm] * 9, out_specs=hbm,
        scratch_shapes=[
            V((4, 8, 64, D), bf), V((2, 321, 1024), bf), V((2, 321, 1024), bf),
            V((3, 128, 256), jnp.uint32), V((R, 64, 128), jnp.uint32), V((R, 64, 128), jnp.uint32),
            V((4, 128, 128), f32), V((4, R, 128), f32),
            V((3, 32, 64, 128), f32), V((3, 32, 64, 128), f32),
            V((3, 2112, 128), jnp.uint32),
            V((2, S_, D), bf), V((2, 4, 128, 128), bf), V((2, 4, 128, 128), bf), V((3, 128, D), f32), V((3, 128, D), bf),
            V((16, 2, 160, 128), jnp.uint32),
            V((S_, D), bf), V((D, 3 * D), bf), V((D, D), bf), V((2 * D, D), bf),
            V((NB + 2, 128, 1024), bf), V((NB + 2, 1024, 128), bf),
            V((2, D, 128), f32), V((D, 128), f32), V((128, D), bf),
            pltpu.SemaphoreType.DMA((13,)), pltpu.SemaphoreType.DMA((2,)),
        ],
        compiler_params=pltpu.CompilerParams(vmem_limit_bytes=110 * 2**20),
        name='fused',
    )(A_x.reshape(8, 4, 64, D), wrT, wiT, B_x.reshape(S_, D), B_wqkv, B_wo,
      jnp.asarray(RD_U32), jnp.asarray(E_NP), jnp.asarray(CS_NP))
    return out.reshape(1, S_, 2 * D)


@jax.jit
def pallas_concat_heads__spectral_gfnet__sliding_block__prompt_kernel(
    A_x: jax.Array,
    A_w_r: jax.Array,
    A_w_i: jax.Array,
    B_x: jax.Array,
    B_wqkv: jax.Array,
    B_wo: jax.Array,
):
    return run(A_x, A_w_r, A_w_i, B_x, B_wqkv, B_wo, UNR=5, LAG=10, WU0=12, NWU=4, MB0=6)
```

```python
import numpy as np
import jax
import jax.numpy as jnp
from jax import lax
import jax.experimental.pallas as pl
import jax.experimental.pallas.tpu as pltpu

bf = jnp.bfloat16
f32 = jnp.float32
u32 = jnp.uint32
S_ = 2048
D = 640
NB = 16
NH = 32
R = 32
QSCALE = float((20 ** -0.5) * np.log2(np.e))
NEG = -1e30
SIG = float(2.0 / (S_ * D))
C1, C2 = float(np.cos(2 * np.pi / 5)), float(np.cos(4 * np.pi / 5))
S1, S2 = float(np.sin(2 * np.pi / 5)), float(np.sin(4 * np.pi / 5))

LAG = 10
UNROLL = 5


def _consts():
    n2 = np.arange(128)[:, None].astype(np.float64)
    m_ = np.arange(32)

    def gmat(r1, r2):
        l = np.concatenate([r1 + 10 * m_, r1 + 5 + 10 * m_, r2 + 10 * m_, r2 + 5 + 10 * m_]).astype(np.float64)[None, :]
        c = np.cos(2 * np.pi * n2 * l / D)
        s = np.sin(2 * np.pi * n2 * l / D)
        sg = np.concatenate([np.ones(64), -np.ones(64)])[None, :]
        return np.block([[c, -s], [sg * s, sg * c]])

    g = np.zeros((3, 256, 256))
    g[0] = gmat(1, 4)
    g[1] = gmat(2, 3)
    l0 = np.concatenate([10 * m_, 5 + 10 * m_]).astype(np.float64)[None, :]
    g0 = np.concatenate([np.cos(2 * np.pi * n2 * l0 / D), -np.sin(2 * np.pi * n2 * l0 / D)], axis=1)
    g0[:, 64] = np.cos(np.pi * n2[:, 0])
    g[2, :128, :128] = g0
    perm = np.array([64 * ((r % 16) // 8) + 8 * (r // 16) + (r % 8) for r in range(128)])
    pre = np.array([16 * (r // 16) + 2 * (r % 8) + ((r % 16) // 8) for r in range(128)])
    s2f = perm % 64
    s2i = perm[pre] % 64
    k1 = np.arange(R)[:, None]
    ang = lambda s2: 2 * np.pi * ((k1 * s2[None, :]) % S_) / S_
    cs = np.stack([np.cos(ang(s2f)), -np.sin(ang(s2f)), np.cos(ang(s2i)), -np.sin(ang(s2i))])
    gb = g.astype(np.float32).astype(jnp.bfloat16).view(np.uint16).astype(np.uint32)
    g_u32 = (gb[:, 0::2, :] | (gb[:, 1::2, :] << 16)).astype(np.uint32)
    return g_u32, cs.astype(np.float32)


G_U32, CS_NP = _consts()


def _radix5_fwd(x):
    t1, t2 = x[1] + x[4], x[2] + x[3]
    t3, t4 = x[1] - x[4], x[2] - x[3]
    a0 = x[0] + t1 + t2
    a1 = x[0] + C1 * t1 + C2 * t2
    a2 = x[0] + C2 * t1 + C1 * t2
    b1 = -(S1 * t3 + S2 * t4)
    b2 = S1 * t4 - S2 * t3
    return [a0, a1, b1, a2, b2]


def _radix5_inv(q0, q1r, q1i, q2r, q2i):
    q0s = SIG * q0
    t1 = q0s + (SIG * C1) * q1r + (SIG * C2) * q2r
    t2 = q0s + (SIG * C2) * q1r + (SIG * C1) * q2r
    u1 = (SIG * S1) * q1i + (SIG * S2) * q2i
    u2 = (SIG * S2) * q1i - (SIG * S1) * q2i
    return [SIG * (q0 + q1r + q2r), t1 - u1, t2 - u2, t2 + u2, t1 + u1]


def _cmul_const(v, ang):
    re, im = v
    c, s = float(np.cos(ang)), float(np.sin(ang))
    eps = 1e-12
    if abs(s) < eps:
        return (re, im) if c > 0 else (-re, -im)
    if abs(c) < eps:
        return (-im, re) if s > 0 else (im, -re)
    if abs(abs(c) - abs(s)) < eps:
        h = abs(c)
        if c > 0 and s > 0:
            return ((re - im) * h, (re + im) * h)
        if c > 0 and s < 0:
            return ((re + im) * h, (im - re) * h)
        if c < 0 and s > 0:
            return ((re + im) * (-h), (re - im) * h)
        return ((im - re) * h, (re + im) * (-h))
    return (re * c - im * s, re * s + im * c)


def _fft(xs, sign):
    n = len(xs)
    if n == 1:
        return xs
    ev = _fft(xs[0::2], sign)
    od = _fft(xs[1::2], sign)
    out = [None] * n
    for k in range(n // 2):
        er, ei = ev[k]
        orr, oi = od[k]
        if 4 * k == n:
            if sign < 0:
                out[k] = (er + oi, ei - orr)
                out[k + n // 2] = (er - oi, ei + orr)
            else:
                out[k] = (er - oi, ei + orr)
                out[k + n // 2] = (er + oi, ei - orr)
        else:
            tr, ti = _cmul_const((orr, oi), sign * 2 * np.pi * k / n)
            out[k] = (er + tr, ei + ti)
            out[k + n // 2] = (er - tr, ei - ti)
    return out


def _radix4(v, sign):
    (ar, ai), (br, bi), (cr, ci), (dr, di) = v
    s0r, s0i = ar + cr, ai + ci
    s1r, s1i = ar - cr, ai - ci
    s2r, s2i = br + dr, bi + di
    s3r, s3i = br - dr, bi - di
    o0 = (s0r + s2r, s0i + s2i)
    o2 = (s0r - s2r, s0i - s2i)
    if sign < 0:
        o1 = (s1r + s3i, s1i - s3r)
        o3 = (s1r - s3i, s1i + s3r)
    else:
        o1 = (s1r - s3i, s1i + s3r)
        o3 = (s1r + s3i, s1i - s3r)
    return [o0, o1, o2, o3]


_NT = (((1,), (1,)), ((), ()))


def _kernel(ax_h, wr_h, wi_h, bx_h, wqkv_h, wo_h, g_h, cs_h, out_h,
            xa, wr_v, wi_v, g_v, mf_v, mi_v, e_v, cs_v, PR, PI, WW, Y, YS, ZF, XL, WU,
            xb, wqkv_v, wo_v, wT, KP, VT, QT, OT, OS, sems, osem):
    cp = lambda s_, d_, i: pltpu.make_async_copy(s_, d_, sems.at[i])
    cp_g = cp(g_h, g_v, 0)
    cp_xa = [cp(ax_h.at[:, i], xa.at[i], 1 + i) for i in range(4)]
    cp_wg = [[cp(h_.at[:, pl.ds(1024 * g_, 1024)], v_.at[g_], 5 + g_) for (h_, v_) in ((wr_h, wr_v), (wi_h, wi_v))]
             for g_ in range(2)]
    cp_cs = cp(cs_h, cs_v, 7)
    cp_w = cp(wqkv_h, wqkv_v, 8)
    cp_xb = [cp(bx_h.at[pl.ds(0, 256), :], xb.at[pl.ds(0, 256), :], 8),
             cp(bx_h.at[pl.ds(256, 1792), :], xb.at[pl.ds(256, 1792), :], 9)]
    cp_wo = cp(wo_h, wo_v, 9)
    for c_ in (cp_xa[0], cp_g, cp_cs, cp_xa[1], cp_xa[2], cp_xa[3], *cp_wg[0], *cp_wg[1],
               cp_w, cp_xb[0], cp_wo, cp_xb[1]):
        c_.start()

    tb = lambda v: pltpu.bitcast(v, bf)
    HI = jnp.uint32(0xffff0000)

    def pk2(a_, b_):
        ua = pltpu.bitcast(a_, u32) + jnp.uint32(0x8000)
        ub = pltpu.bitcast(b_, u32) + jnp.uint32(0x8000)
        return (ua >> 16) | (ub & HI)

    def upk(w_, i_):
        return pltpu.bitcast(w_ << 16, f32) if i_ == 0 else pltpu.bitcast(w_ & HI, f32)

    sub8 = lax.broadcasted_iota(jnp.int32, (8, 128), 0)
    col8 = lax.broadcasted_iota(jnp.int32, (8, 128), 1)
    lane = lax.broadcasted_iota(jnp.int32, (128, 128), 1)
    lane64 = lax.broadcasted_iota(jnp.int32, (64, 128), 1)
    lane32 = lax.broadcasted_iota(jnp.int32, (32, 128), 1)

    def init_pads():
        lane_k = lax.broadcasted_iota(jnp.int32, (128, 1024), 1)
        kpad = jnp.where((lane_k % 128) == 127, NEG, 0.0).astype(bf)
        KP[0] = kpad
        KP[1] = kpad
        VT[0] = jnp.zeros((1024, 128), bf)
        VT[1] = jnp.zeros((1024, 128), bf)
        OT[...] = jnp.zeros(OT.shape, f32)

    def proj_k(b, xblk):
        kf = jnp.dot(xblk, wqkv_v[:, 640:1280], preferred_element_type=f32)
        for g in range(8):
            off = 80 * g
            t = off // 128
            sh = off % 128
            s0 = kf[:, 128 * t:128 * t + 128]
            if sh:
                s0 = pltpu.roll(s0, 128 - sh, 1)
            if sh + 80 > 128:
                s1 = pltpu.roll(kf[:, 128 * (t + 1):128 * (t + 2)], 128 - sh, 1)
                tile = jnp.where(lane < 128 - sh, s0, jnp.where(lane < 80, s1, 0.0))
            else:
                tile = jnp.where(lane < 80, s0, 0.0)
            KP[b + 2, :, 128 * g:128 * g + 128] = tile.astype(bf)

    def proj_qv(b, xblk, slot):
        nt = lambda lo, n: lax.dot_general(wT[lo:lo + n, :], xblk, _NT, preferred_element_type=f32)
        QT[slot, 0:320, :] = nt(0, 320) * QSCALE
        QT[slot, 320:640, :] = nt(320, 320) * QSCALE
        vv = jnp.concatenate([nt(640, 320), nt(960, 320)], axis=0)
        cA = jnp.where(sub8 == 4, 1.0, 0.0).astype(f32)
        cB = jnp.where(sub8 == 0, 1.0, 0.0).astype(f32)
        z8 = jnp.zeros((8, 128), f32)
        for p in range(16):
            v = [vv[40 * p + 8 * i: 40 * p + 8 * i + 8] for i in range(5)]
            blk = jnp.concatenate([v[0], v[1], jnp.where(sub8 < 4, v[2], cA), z8,
                                   jnp.where(sub8 >= 4, v[2], cB), v[3], v[4], z8], axis=0)
            VT[b + 2, 64 * p:64 * p + 64, :] = blk.astype(bf)

    def q_rows(h, slot):
        g, i = h // 4, h % 4
        a = (20 * i) // 16
        q = QT[slot, g * 80 + 16 * a: g * 80 + 16 * a + 32, :]
        r = lax.broadcasted_iota(jnp.int32, (32, 128), 0) + 16 * a
        return a, q, (r >= 20 * i) & (r < 20 * i + 20)

    def q_rows_shift(h, slot):
        g, i = h // 4, h % 4
        o_ = (20 * i) % 8
        q2 = QT[slot, g * 80 + 20 * i - o_: g * 80 + 20 * i - o_ + 24, :]
        r2 = lax.broadcasted_iota(jnp.int32, (24, 128), 0)
        c2 = lax.broadcasted_iota(jnp.int32, (24, 128), 1)
        return q2, (r2 >= o_) & (r2 < o_ + 20), c2

    def build_w(h, slot):
        a, q, rm = q_rows(h, slot)
        parts = []
        if a > 0:
            parts.append(jnp.zeros((16 * a, 128), f32))
        parts.append(jnp.where(rm, q, 0.0))
        parts.append(jnp.zeros((120 - 16 * a - 32, 128), f32))
        parts.append(jnp.where(sub8 == 7, 1.0, 0.0).astype(f32))
        return jnp.concatenate(parts, axis=0).astype(bf)

    def build_wd(h, slot):
        a, q, rm = q_rows(h, slot)
        c = lax.broadcasted_iota(jnp.int32, (32, 128), 1)
        q2, rm2, c2 = q_rows_shift(h, slot)
        parts = []
        if a > 0:
            parts.append(jnp.zeros((16 * a, 128), f32))
        parts.append(jnp.where(rm & (c < 64), q, 0.0))
        if 80 - 16 * a - 32 > 0:
            parts.append(jnp.zeros((80 - 16 * a - 32, 128), f32))
        parts.append(jnp.where(rm2 & (c2 >= 64), q2, 0.0))
        parts.append(jnp.zeros((16, 128), f32))
        parts.append(jnp.where((sub8 == 7) & (col8 < 64), 1.0, 0.0).astype(f32))
        return jnp.concatenate(parts, axis=0).astype(bf)

    def build_wd2(h, slot):
        q2, rm2, c2 = q_rows_shift(h, slot)
        parts = [jnp.where(rm2 & (c2 >= 32 * s_) & (c2 < 32 * s_ + 32), q2, 0.0) for s_ in range(4)]
        parts.append(jnp.zeros((24, 128), f32))
        parts.append(jnp.where((sub8 == 7) & ((col8 // 32) % 2 == 0), 1.0, 0.0).astype(f32))
        return jnp.concatenate(parts, axis=0).astype(bf)

    def qk_dot(b, h, slot, order):
        g, i = h // 4, h % 4
        lo, hi = g * 128, (g + 1) * 128
        o_ = (20 * i) % 8
        w = build_w(h, slot)
        kt = jnp.concatenate([KP[b + 2, 0:32, lo:hi], KP[b, 96:128, lo:hi], KP[b + 1, :, lo:hi]], axis=0)
        rl = pltpu.roll(KP[b + 2, 32:96, lo:hi], 80 + o_ - 20 * i, 1)
        ld = jnp.where((lane64 >= 80) & (lane64 < 104), rl, KP[b, 32:96, lo:hi])
        srcs = [KP[b, 0:32, lo:hi], KP[b + 2, 32:64, lo:hi], KP[b, 64:96, lo:hi], KP[b + 2, 96:128, lo:hi]]
        l2 = None
        for s_ in range(4):
            d_ = 24 * s_ + o_
            shift = (d_ - 20 * i) % 128
            v = pltpu.roll(srcs[s_], shift, 1) if shift else srcs[s_]
            if s_ == 0:
                l2 = jnp.where(lane32 == 127, srcs[0], v) if shift else v
            else:
                l2 = jnp.where((lane32 >= d_) & (lane32 < d_ + 20), v, l2)
        res = {}
        for ch in order:
            if ch == 'm':
                res[ch] = jnp.dot(kt, w, preferred_element_type=f32)
            elif ch == 'c':
                res[ch] = jnp.dot(ld, build_wd(h, slot), preferred_element_type=f32)
            else:
                res[ch] = jnp.dot(l2, build_wd2(h, slot), preferred_element_type=f32)
        return res['m'], res['c'], res['d']

    def max_stage(sd):
        si, cb, dg = sd
        mx = None
        scs = []
        for a in range(16):
            tri = sub8 + 8 * a > col8
            d_ = dg[8 * (a % 4):8 * (a % 4) + 8]
            if a < 4:
                sc = jnp.where(tri, d_, si[8 * a:8 * a + 8])
            elif a < 8:
                sc = jnp.where((col8 >= 32) & (col8 < 64) & jnp.logical_not(tri), d_, cb[8 * a - 32:8 * a - 24])
            elif a < 12:
                sc = jnp.where((col8 >= 64) & (col8 < 96) & tri, d_, cb[8 * a - 32:8 * a - 24])
            else:
                sc = jnp.where(tri, si[8 * a - 64:8 * a - 56], d_)
            scs.append(sc)
            mx = sc if mx is None else jnp.maximum(mx, sc)
        sm = si[64:192]
        for a in range(16):
            mx = jnp.maximum(mx, sm[8 * a:8 * a + 8])
        mx = jnp.max(mx, axis=0, keepdims=True)
        return (jnp.concatenate(scs, axis=0), sm, mx)

    def exp_pv(b, h, st):
        sc, sm, m = st
        row = lax.broadcasted_iota(jnp.int32, (128, 128), 0)
        pc = jnp.exp2(sc - m)
        pm = jnp.exp2(sm - m)
        msk = row > lane
        pu = jnp.where(msk, pc, 0.0)
        pl_ = jnp.where(msk, 0.0, pc)
        pall = jnp.concatenate([pu, pm, pl_], axis=0).astype(bf)
        vt = jnp.concatenate([VT[b + t, 32 * h:32 * h + 32, :] for t in range(3)], axis=1)
        o = jnp.dot(vt, pall, preferred_element_type=f32)
        l = o[20:21, :] if h % 2 == 0 else o[0:1, :]
        r = pltpu.reciprocal(l, approx=False)
        return o[0:24] * r

    def fin_o():
        for kt in range(5):
            OS[:, 128 * kt:128 * kt + 128] = OT[128 * kt:128 * kt + 128, :].T.astype(bf)

    def outproj(bprev):
        y = jnp.dot(OS[...], wo_v[...], preferred_element_type=f32)
        Y[1, pl.ds(pl.multiple_of(bprev * 128, 128), 128), :] = y.astype(bf)

    def out_copy(bb, half):
        rows = pl.ds(pl.multiple_of(bb * 128, 128), 128)
        return pltpu.make_async_copy(Y.at[half, rows, :],
                                     out_h.at[rows, pl.ds(pl.multiple_of(640 * half, 128), 640)], osem.at[0])

    units = [(a, j) for a in range(4) for j in range(4)]
    bsplit = [(0, 1, 2), (3, 4, 5), (6, 7)]

    def r5_fwd(u, bs):
        a, j = units[u]
        for b in bs:
            xs = [xa[a, b, 16 * j:16 * j + 16, 128 * t:128 * t + 128].astype(f32) for t in range(5)]
            o = _radix5_fwd(xs)
            for t in range(5):
                XL[u % 3, 16 * b:16 * b + 16, 128 * t:128 * t + 128] = o[t].astype(bf)

    def dfwd_dot(u, n):
        if n == 0:
            r_ = jnp.dot(XL[u % 3, :, 128:384], tb(g_v[0]), preferred_element_type=f32)
            return (r_[:, 0:128], r_[:, 128:256])
        if n == 1:
            r_ = jnp.dot(XL[u % 3, :, 384:640], tb(g_v[1]), preferred_element_type=f32)
            return (r_[:, 0:128], r_[:, 128:256])
        return jnp.dot(XL[u % 3, :, 0:128], tb(g_v[2, 0:64, 0:128]), preferred_element_type=f32)

    def fwd_fft_unit(a, p, j, t):
        for hh in range(2):
            xs = []
            for b in range(8):
                r = slice(16 * b + 8 * hh, 16 * b + 8 * hh + 8)
                if p < 2:
                    re = t[0][r]
                    im = t[1][r]
                else:
                    m = t[r]
                    re = jnp.where(col8 <= 64, m, 0.0)
                    im = jnp.where((col8 >= 1) & (col8 < 64), pltpu.roll(m, 64, 1), 0.0)
                xs.append((re, im))
            ys = _fft(xs, -1)
            rr = slice(16 * j + 8 * hh, 16 * j + 8 * hh + 8)
            for kp in range(8):
                y = _cmul_const(ys[kp], -2 * np.pi * a * kp / 32)
                PR[p, a * 8 + kp, rr, :] = y[0]
                PI[p, a * 8 + kp, rr, :] = y[1]

    def wretile(c):
        cs = slice(128 * (c % 8), 128 * (c % 8) + 128)
        WU[c, 0] = pltpu.bitcast(wr_v[c // 8, 0:320, cs], u32)
        WU[c, 1] = pltpu.bitcast(wi_v[c // 8, 0:320, cs], u32)

    def wprep1(c, p):
        def rows(rho):
            sl = pl.ds(rho // 2, 32, stride=5)
            a_ = upk(WU[c, 0, sl, :], rho % 2)
            b_ = upk(WU[c, 1, sl, :], rho % 2)
            if rho == 0:
                r32 = lax.broadcasted_iota(jnp.int32, (32, 128), 0)
                a_ = jnp.where(r32 == 0, 0.5 * a_, a_)
                b_ = jnp.where(r32 == 0, 0.5 * b_, b_)
            return (pltpu.bitcast(a_, u32) >> 16) | pltpu.bitcast(b_, u32)
        if p < 2:
            r1, r2 = (1, 4) if p == 0 else (2, 3)
            w = jnp.concatenate([rows(r1), rows(r1 + 5), rows(r2), rows(r2 + 5)], axis=0)
        else:
            cs = slice(128 * (c % 8), 128 * (c % 8) + 128)
            a_ = jnp.where(sub8 == 0, 0.5 * jnp.broadcast_to(wr_v[c // 8, 320:321, cs].astype(f32), (8, 128)), 0.0)
            b_ = jnp.where(sub8 == 0, 0.5 * jnp.broadcast_to(wi_v[c // 8, 320:321, cs].astype(f32), (8, 128)), 0.0)
            nyq = (pltpu.bitcast(a_, u32) >> 16) | pltpu.bitcast(b_, u32)
            w = jnp.concatenate([rows(0), rows(5), nyq, jnp.zeros((56, 128), u32)], axis=0)
        w = w.T
        for q in range(4):
            WW[p, pl.ds(33 * (4 * c + q), 32), :] = w[32 * q:32 * q + 32]

    def build_e():
        comp = lambda v: ((v % 16) // 8, 8 * (v // 16) + v % 8)
        pre_ = lambda v: 16 * (v // 16) + 2 * (v % 8) + (v % 16) // 8
        for blk in range(16):
            r = sub8 + 8 * blk
            for form in range(2):
                (cr, k2_), (cc, s2_) = (comp(pre_(r)), comp(col8)) if form == 0 else (comp(r), comp(pre_(col8)))
                th = ((k2_ * s2_) % 64).astype(f32) * float(2 * np.pi / 64)
                cs_, sn_ = jnp.cos(th), jnp.sin(th)
                same = cr == cc
                e_v[2 * form, 8 * blk:8 * blk + 8, :] = jnp.where(same, cs_, jnp.where(cr == 1, -sn_, sn_))
                e_v[2 * form + 1, 8 * blk:8 * blk + 8, :] = jnp.where(same, sn_, jnp.where(cr == 1, cs_, -cs_))

    def mbuild(k1):
        cf = jnp.broadcast_to(cs_v[0, k1:k1 + 1, :], (8, 128))
        sf = jnp.broadcast_to(cs_v[1, k1:k1 + 1, :], (8, 128))
        for v in range(8):
            lo = e_v[0, 16 * v:16 * v + 8, :] * cf + e_v[1, 16 * v:16 * v + 8, :] * sf
            hi = e_v[0, 16 * v + 8:16 * v + 16, :] * cf + e_v[1, 16 * v + 8:16 * v + 16, :] * sf
            mf_v[k1, 8 * v:8 * v + 8, :] = pk2(lo, hi)
        ci = jnp.broadcast_to(cs_v[2, k1:k1 + 1, :], (8, 128))
        si = jnp.broadcast_to(cs_v[3, k1:k1 + 1, :], (8, 128))
        nn = jnp.concatenate([e_v[2, 8 * r:8 * r + 8, :] * ci + e_v[3, 8 * r:8 * r + 8, :] * si
                              for r in range(16)], axis=0).T
        for v in range(8):
            mi_v[k1, 8 * v:8 * v + 8, :] = pk2(nn[16 * v:16 * v + 8], nn[16 * v + 8:16 * v + 16])

    def pre(kp, p):
        tl = [[] for _ in range(4)]
        for g in range(8):
            v = [(PR[p, a * 8 + kp, 8 * g:8 * g + 8, :], PI[p, a * 8 + kp, 8 * g:8 * g + 8, :]) for a in range(4)]
            ts = _radix4(v, -1)
            for kk in range(4):
                tl[kk] += [ts[kk][0], ts[kk][1]]
        return [jnp.concatenate(t_, axis=0).astype(bf) for t_ in tl]

    def fwd(kp, ts):
        return [jnp.dot(tb(mf_v[kp + 8 * kk]), ts[kk], preferred_element_type=f32) for kk in range(4)]

    def mid(u, kp, p, xs):
        for g in range(8):
            for kk in range(4):
                k1 = kp + 8 * kk
                x = xs[kk]
                xr, xi = x[16 * g:16 * g + 8], x[16 * g + 8:16 * g + 16]
                ww = WW[p, pl.ds(k1 + 33 * 8 * g, 8, stride=33), :]
                wr = upk(ww, 0)
                wi = upk(ww, 1)
                YS[u % 2, kk, 16 * g:16 * g + 16, :] = jnp.concatenate(
                    [xr * wr - xi * wi, xr * wi + xi * wr], axis=0).astype(bf)

    def inv(u, kp):
        return [jnp.dot(tb(mi_v[kp + 8 * kk]), YS[u % 2, kk], preferred_element_type=f32) for kk in range(4)]

    def post(kp, p, outs):
        for g in range(8):
            v = [(o[16 * g:16 * g + 8], o[16 * g + 8:16 * g + 16]) for o in outs]
            r = _radix4(v, +1)
            for a in range(4):
                PR[p, a * 8 + kp, 8 * g:8 * g + 8, :] = r[a][0]
                PI[p, a * 8 + kp, 8 * g:8 * g + 8, :] = r[a][1]

    def inv_unit_p(u, p):
        a, j = units[u]
        for hh in range(2):
            rr = slice(16 * j + 8 * hh, 16 * j + 8 * hh + 8)
            xs = []
            for kp in range(8):
                v = (PR[p, a * 8 + kp, rr, :], PI[p, a * 8 + kp, rr, :])
                xs.append(_cmul_const(v, 2 * np.pi * a * kp / 32))
            zs = _fft(xs, +1)
            for b in range(8):
                r = slice(16 * b + 8 * hh, 16 * b + 8 * hh + 8)
                zr, zi = zs[b]
                if p == 2:
                    ZF[u % 3, r, 0:128] = jnp.where(col8 <= 64, zr, pltpu.roll(zi, 64, 1))
                elif p == 0:
                    ZF[u % 3, r, 128:256] = zr
                    ZF[u % 3, r, 256:384] = zi
                else:
                    ZF[u % 3, r, 384:512] = zr
                    ZF[u % 3, r, 512:640] = zi

    def dinv_dot(u, n):
        if n == 0:
            return lax.dot_general(ZF[u % 3, :, 128:384].astype(bf), tb(g_v[0]), _NT, preferred_element_type=f32)
        if n == 1:
            return lax.dot_general(ZF[u % 3, :, 384:640].astype(bf), tb(g_v[1]), _NT, preferred_element_type=f32)
        return lax.dot_general(ZF[u % 3, :, 0:128].astype(bf), tb(g_v[2, 0:64, 0:128]), _NT, preferred_element_type=f32)

    def r5_inv(u, qs, bs):
        a, j = units[u]
        q1, q2, q0 = qs
        for b in bs:
            r = slice(16 * b, 16 * b + 16)
            ys = _radix5_inv(q0[r], q1[r, 0:128], q1[r, 128:256], q2[r, 0:128], q2[r, 128:256])
            for t in range(5):
                Y[0, pl.ds(64 * (a + 4 * b) + 16 * j, 16), 128 * t:128 * t + 128] = ys[t].astype(bf)

    def wt_job(i, half):
        base = 0 if half == 0 else 1280
        wT[640 * half + 128 * i:640 * half + 128 * i + 128, :] = wqkv_v[:, base + 128 * i:base + 128 * i + 128].T

    a_out = pltpu.make_async_copy(Y.at[0, pl.ds(128, S_ - 128), :],
                                  out_h.at[pl.ds(128, S_ - 128), pl.ds(0, 640)], osem.at[1])

    build_e()
    init_pads()
    cp_xa[0].wait()
    wjobs = [(c, p_) for c in range(16) for p_ in range(3)]
    r5_fwd(0, range(8))
    r5_fwd(1, range(8))
    cp_g.wait()
    cp_cs.wait()
    dres = {}
    for q in range(48 + 1):
        qq = q - 1
        if qq >= 0 and qq % 3 == 0:
            u = qq // 3
            if u + 2 < 16 and units[u + 2][1] == 0:
                cp_xa[units[u + 2][0]].wait()
            if u == 12:
                for c_ in cp_wg[0]:
                    c_.wait()
        if q < 48:
            dres[q] = dfwd_dot(q // 3, q % 3)
        if qq < 0:
            continue
        u, n = qq // 3, qq % 3
        if u + 2 < 16:
            r5_fwd(u + 2, bsplit[n])
        if 12 <= u < 16:
            k_ = (u - 12) * 3 + n
            if k_ == 0:
                for c_i in range(8):
                    wretile(c_i)
            for jb in wjobs[2 * k_:2 * k_ + 2]:
                wprep1(*jb)
        if 6 <= qq < 6 + R:
            mbuild(qq - 6)
        fwd_fft_unit(u // 4, n, u % 4, dres.pop(qq))
    for c_ in cp_wg[1]:
        c_.wait()
    for c_i in range(8, 16):
        wretile(c_i)
    for c_i in range(8, 16):
        wprep1(c_i, 0)
    us = [(kp, p) for p in range(3) for kp in range(8)]
    xr_ = {}
    or_ = {}
    tl_ = {0: pre(*us[0])}
    for t in range(24 + 2):
        if t < 24:
            xr_[t] = fwd(us[t][0], tl_.pop(t))
        if t >= 2:
            post(*us[t - 2], or_.pop(t - 2))
        if t + 1 < 24:
            tl_[t + 1] = pre(*us[t + 1])
        if 1 <= t <= 24:
            or_[t - 1] = inv(t - 1, us[t - 1][0])
        if t < 16:
            wprep1(8 + t % 8, 1 + t // 8)
        if t < 24:
            mid(t, *us[t], xr_.pop(t))
    cp_w.wait()
    cp_xb[0].wait()
    x0 = xb[0:128, :]
    proj_k(0, x0)
    for p in range(3):
        inv_unit_p(0, p)
    for p in range(3):
        inv_unit_p(1, p)
    qres = {}
    for u in range(16 + 1):
        for n in range(3):
            if u < 16:
                qres[(u, n)] = dinv_dot(u, n)
            if u + 2 < 16:
                inv_unit_p(u + 2, n)
            if u >= 1:
                r5_inv(u - 1, [qres[(u - 1, 0)], qres[(u - 1, 1)], qres[(u - 1, 2)]], bsplit[n])
            if n == 2 and 1 <= u < 11:
                wt_job((u - 1) // 2, (u - 1) % 2)
        if u == 15:
            proj_qv(0, x0, 0)
    a_out.start()
    cp_wo.wait()
    cp_xb[1].wait()

    def step(b, last):
        slot = b % 2
        bp = b - 1 if last else jnp.maximum(b - 1, 0)
        order = 'dcm' if last else 'dmc'
        t_out = NH + 1 if last else 2
        dots = {}
        sts = {}
        outs = {}
        if not last:
            bn = b + 1
        for t in range(NH + LAG):
            if t < NH:
                dots[t] = qk_dot(b, t, slot, order)
            if t == 0:
                fin_o()
            if t == t_out:
                outproj(bp)
            if 0 <= t - 2 < NH:
                sts[t - 2] = max_stage(dots.pop(t - 2))
            if t == NH and not last:
                xn = xb[pl.ds(pl.multiple_of(bn * 128, 128), 128), :]
                proj_k(bn, xn)
            if 0 <= t - LAG < NH:
                h = t - LAG
                outs[h] = exp_pv(b, h, sts.pop(h))
                if h % 2 == 1:
                    A = outs.pop(h - 1)
                    B = outs.pop(h)
                    p = h // 2
                    OT[40 * p:40 * p + 40, :] = jnp.concatenate(
                        [A[0:16], jnp.where(sub8 < 4, A[16:24], B[0:8]), B[8:24]], axis=0)
        if last:
            out_copy(bp, 1).start()
        else:
            proj_qv(bn, xn, 1 - slot)
            out_copy(bp, jnp.minimum(b, 1)).start()

    def body(b, carry):
        step(b, False)
        return carry

    lax.fori_loop(0, NB - 1, body, 0, unroll=UNROLL)
    step(NB - 1, True)
    fin_o()
    lastc = []
    r0 = (NB - 1) * 128
    for n in range(5):
        y_ = jnp.dot(OS[...], wo_v[:, 128 * n:128 * n + 128], preferred_element_type=f32)
        Y[1, r0:r0 + 128, 128 * n:128 * n + 128] = y_.astype(bf)
        c_ = pltpu.make_async_copy(Y.at[1, pl.ds(r0, 128), pl.ds(128 * n, 128)],
                                   out_h.at[pl.ds(r0, 128), pl.ds(640 + 128 * n, 128)], osem.at[2])
        c_.start()
        lastc.append(c_)
    a_out.wait()
    for i in range(NB):
        out_copy(0, 1).wait()
    for c_ in lastc:
        c_.wait()


@jax.jit
def pallas_concat_heads__spectral_gfnet__sliding_block__prompt_kernel(
    A_x: jax.Array,
    A_w_r: jax.Array,
    A_w_i: jax.Array,
    B_x: jax.Array,
    B_wqkv: jax.Array,
    B_wo: jax.Array,
):
    hbm = pl.BlockSpec(memory_space=pltpu.HBM)
    V = pltpu.VMEM
    out = pl.pallas_call(
        _kernel,
        out_shape=jax.ShapeDtypeStruct((S_, 2 * D), bf),
        in_specs=[hbm] * 8,
        out_specs=hbm,
        scratch_shapes=[
            V((4, 8, 64, D), bf), V((2, 321, 1024), bf), V((2, 321, 1024), bf),
            V((3, 128, 256), u32), V((R, 64, 128), u32), V((R, 64, 128), u32),
            V((4, 128, 128), f32), V((4, R, 128), f32),
            V((3, 32, 64, 128), f32), V((3, 32, 64, 128), f32),
            V((3, 2112, 128), u32),
            V((2, S_, D), bf), V((2, 4, 128, 128), bf), V((3, 128, D), f32), V((3, 128, D), bf),
            V((16, 2, 160, 128), u32),
            V((S_, D), bf), V((D, 3 * D), bf), V((D, D), bf), V((2 * D, D), bf),
            V((NB + 2, 128, 1024), bf), V((NB + 2, 1024, 128), bf),
            V((2, D, 128), f32), V((D, 128), f32), V((128, D), bf),
            pltpu.SemaphoreType.DMA((10,)), pltpu.SemaphoreType.DMA((3,)),
        ],
        compiler_params=pltpu.CompilerParams(vmem_limit_bytes=110 * 2**20),
        name='fused',
    )(A_x.reshape(8, 4, 64, D), A_w_r.T, A_w_i.T, B_x.reshape(S_, D), B_wqkv, B_wo,
      jnp.asarray(G_U32), jnp.asarray(CS_NP))
    return out.reshape(1, S_, 2 * D)
```

```python
import numpy as np
import jax
import jax.numpy as jnp
from jax import lax
import jax.experimental.pallas as pl
import jax.experimental.pallas.tpu as pltpu

bf = jnp.bfloat16
f32 = jnp.float32
u32 = jnp.uint32
S_ = 2048
D = 640
NB = 16
NH = 32
R = 32
QSCALE = float((20 ** -0.5) * np.log2(np.e))
NEG = -1e30
SIG = float(2.0 / (S_ * D))
C1, C2 = float(np.cos(2 * np.pi / 5)), float(np.cos(4 * np.pi / 5))
S1, S2 = float(np.sin(2 * np.pi / 5)), float(np.sin(4 * np.pi / 5))

LAG = 10
UNROLL = 5


def _consts():
    n2 = np.arange(128)[:, None].astype(np.float64)
    m_ = np.arange(32)

    def gmat(r1, r2):
        l = np.concatenate([r1 + 10 * m_, r1 + 5 + 10 * m_, r2 + 10 * m_, r2 + 5 + 10 * m_]).astype(np.float64)[None, :]
        c = np.cos(2 * np.pi * n2 * l / D)
        s = np.sin(2 * np.pi * n2 * l / D)
        sg = np.concatenate([np.ones(64), -np.ones(64)])[None, :]
        return np.block([[c, -s], [sg * s, sg * c]])

    g = np.zeros((3, 256, 256))
    g[0] = gmat(1, 4)
    g[1] = gmat(2, 3)
    l0 = np.concatenate([10 * m_, 5 + 10 * m_]).astype(np.float64)[None, :]
    g0 = np.concatenate([np.cos(2 * np.pi * n2 * l0 / D), -np.sin(2 * np.pi * n2 * l0 / D)], axis=1)
    g0[:, 64] = np.cos(np.pi * n2[:, 0])
    g[2, :128, :128] = g0
    perm = np.array([64 * ((r % 16) // 8) + 8 * (r // 16) + (r % 8) for r in range(128)])
    pre = np.array([16 * (r // 16) + 2 * (r % 8) + ((r % 16) // 8) for r in range(128)])
    s2f = perm % 64
    s2i = perm[pre] % 64
    k1 = np.arange(R)[:, None]
    ang = lambda s2: 2 * np.pi * ((k1 * s2[None, :]) % S_) / S_
    cs = np.stack([np.cos(ang(s2f)), -np.sin(ang(s2f)), np.cos(ang(s2i)), -np.sin(ang(s2i))])
    gb = g.astype(np.float32).astype(jnp.bfloat16).view(np.uint16).astype(np.uint32)
    g_u32 = (gb[:, 0::2, :] | (gb[:, 1::2, :] << 16)).astype(np.uint32)
    return g_u32, cs.astype(np.float32)


G_U32, CS_NP = _consts()


def _radix5_fwd(x):
    t1, t2 = x[1] + x[4], x[2] + x[3]
    t3, t4 = x[1] - x[4], x[2] - x[3]
    a0 = x[0] + t1 + t2
    a1 = x[0] + C1 * t1 + C2 * t2
    a2 = x[0] + C2 * t1 + C1 * t2
    b1 = -(S1 * t3 + S2 * t4)
    b2 = S1 * t4 - S2 * t3
    return [a0, a1, b1, a2, b2]


def _radix5_inv(q0, q1r, q1i, q2r, q2i):
    q0s = SIG * q0
    t1 = q0s + (SIG * C1) * q1r + (SIG * C2) * q2r
    t2 = q0s + (SIG * C2) * q1r + (SIG * C1) * q2r
    u1 = (SIG * S1) * q1i + (SIG * S2) * q2i
    u2 = (SIG * S2) * q1i - (SIG * S1) * q2i
    return [SIG * (q0 + q1r + q2r), t1 - u1, t2 - u2, t2 + u2, t1 + u1]


def _cmul_const(v, ang):
    re, im = v
    c, s = float(np.cos(ang)), float(np.sin(ang))
    eps = 1e-12
    if abs(s) < eps:
        return (re, im) if c > 0 else (-re, -im)
    if abs(c) < eps:
        return (-im, re) if s > 0 else (im, -re)
    if abs(abs(c) - abs(s)) < eps:
        h = abs(c)
        if c > 0 and s > 0:
            return ((re - im) * h, (re + im) * h)
        if c > 0 and s < 0:
            return ((re + im) * h, (im - re) * h)
        if c < 0 and s > 0:
            return ((re + im) * (-h), (re - im) * h)
        return ((im - re) * h, (re + im) * (-h))
    return (re * c - im * s, re * s + im * c)


def _fft(xs, sign):
    n = len(xs)
    if n == 1:
        return xs
    ev = _fft(xs[0::2], sign)
    od = _fft(xs[1::2], sign)
    out = [None] * n
    for k in range(n // 2):
        er, ei = ev[k]
        orr, oi = od[k]
        if 4 * k == n:
            if sign < 0:
                out[k] = (er + oi, ei - orr)
                out[k + n // 2] = (er - oi, ei + orr)
            else:
                out[k] = (er - oi, ei + orr)
                out[k + n // 2] = (er + oi, ei - orr)
        else:
            tr, ti = _cmul_const((orr, oi), sign * 2 * np.pi * k / n)
            out[k] = (er + tr, ei + ti)
            out[k + n // 2] = (er - tr, ei - ti)
    return out


def _radix4(v, sign):
    (ar, ai), (br, bi), (cr, ci), (dr, di) = v
    s0r, s0i = ar + cr, ai + ci
    s1r, s1i = ar - cr, ai - ci
    s2r, s2i = br + dr, bi + di
    s3r, s3i = br - dr, bi - di
    o0 = (s0r + s2r, s0i + s2i)
    o2 = (s0r - s2r, s0i - s2i)
    if sign < 0:
        o1 = (s1r + s3i, s1i - s3r)
        o3 = (s1r - s3i, s1i + s3r)
    else:
        o1 = (s1r - s3i, s1i + s3r)
        o3 = (s1r + s3i, s1i - s3r)
    return [o0, o1, o2, o3]


_NT = (((1,), (1,)), ((), ()))


def _kernel(ax_h, wr_h, wi_h, bx_h, wqkv_h, wo_h, g_h, cs_h, out_h,
            xa, wr_v, wi_v, g_v, mf_v, mi_v, e_v, cs_v, PR, PI, WW, Y, YS, ZF, XL, WU,
            xb, wqkv_v, wo_v, wT, KP, VT, QT, OT, OS, sems, osem):
    cp = lambda s_, d_, i: pltpu.make_async_copy(s_, d_, sems.at[i])
    cp_g = cp(g_h, g_v, 0)
    cp_xa = [cp(ax_h.at[:, i], xa.at[i], 1 + i) for i in range(4)]
    cp_wg = [[cp(h_.at[:, pl.ds(1024 * g_, 1024)], v_.at[g_], 5 + g_) for (h_, v_) in ((wr_h, wr_v), (wi_h, wi_v))]
             for g_ in range(2)]
    cp_cs = cp(cs_h, cs_v, 7)
    cp_w = cp(wqkv_h, wqkv_v, 8)
    cp_xb = [cp(bx_h.at[pl.ds(0, 256), :], xb.at[pl.ds(0, 256), :], 8),
             cp(bx_h.at[pl.ds(256, 1792), :], xb.at[pl.ds(256, 1792), :], 9)]
    cp_wo = cp(wo_h, wo_v, 9)
    for c_ in (cp_xa[0], cp_g, cp_cs, cp_xa[1], cp_xa[2], cp_xa[3], *cp_wg[0], *cp_wg[1],
               cp_w, cp_xb[0], cp_wo, cp_xb[1]):
        c_.start()

    tb = lambda v: pltpu.bitcast(v, bf)
    HI = jnp.uint32(0xffff0000)

    def pk2(a_, b_):
        ua = pltpu.bitcast(a_, u32) + jnp.uint32(0x8000)
        ub = pltpu.bitcast(b_, u32) + jnp.uint32(0x8000)
        return (ua >> 16) | (ub & HI)

    def upk(w_, i_):
        return pltpu.bitcast(w_ << 16, f32) if i_ == 0 else pltpu.bitcast(w_ & HI, f32)

    sub8 = lax.broadcasted_iota(jnp.int32, (8, 128), 0)
    col8 = lax.broadcasted_iota(jnp.int32, (8, 128), 1)
    lane = lax.broadcasted_iota(jnp.int32, (128, 128), 1)
    lane64 = lax.broadcasted_iota(jnp.int32, (64, 128), 1)
    lane32 = lax.broadcasted_iota(jnp.int32, (32, 128), 1)

    def init_pads():
        lane_k = lax.broadcasted_iota(jnp.int32, (128, 1024), 1)
        kpad = jnp.where((lane_k % 128) == 127, NEG, 0.0).astype(bf)
        KP[0] = kpad
        KP[1] = kpad
        VT[0] = jnp.zeros((1024, 128), bf)
        VT[1] = jnp.zeros((1024, 128), bf)
        OT[...] = jnp.zeros(OT.shape, f32)

    def proj_k(b, xblk):
        kf = jnp.dot(xblk, wqkv_v[:, 640:1280], preferred_element_type=f32)
        for g in range(8):
            off = 80 * g
            t = off // 128
            sh = off % 128
            s0 = kf[:, 128 * t:128 * t + 128]
            if sh:
                s0 = pltpu.roll(s0, 128 - sh, 1)
            if sh + 80 > 128:
                s1 = pltpu.roll(kf[:, 128 * (t + 1):128 * (t + 2)], 128 - sh, 1)
                tile = jnp.where(lane < 128 - sh, s0, jnp.where(lane < 80, s1, 0.0))
            else:
                tile = jnp.where(lane < 80, s0, 0.0)
            KP[b + 2, :, 128 * g:128 * g + 128] = tile.astype(bf)

    def proj_qv(b, xblk, slot):
        nt = lambda lo, n: lax.dot_general(wT[lo:lo + n, :], xblk, _NT, preferred_element_type=f32)
        QT[slot, 0:320, :] = nt(0, 320) * QSCALE
        QT[slot, 320:640, :] = nt(320, 320) * QSCALE
        vv = jnp.concatenate([nt(640, 320), nt(960, 320)], axis=0)
        cA = jnp.where(sub8 == 4, 1.0, 0.0).astype(f32)
        cB = jnp.where(sub8 == 0, 1.0, 0.0).astype(f32)
        z8 = jnp.zeros((8, 128), f32)
        for p in range(16):
            v = [vv[40 * p + 8 * i: 40 * p + 8 * i + 8] for i in range(5)]
            blk = jnp.concatenate([v[0], v[1], jnp.where(sub8 < 4, v[2], cA), z8,
                                   jnp.where(sub8 >= 4, v[2], cB), v[3], v[4], z8], axis=0)
            VT[b + 2, 64 * p:64 * p + 64, :] = blk.astype(bf)

    def q_rows(h, slot):
        g, i = h // 4, h % 4
        a = (20 * i) // 16
        q = QT[slot, g * 80 + 16 * a: g * 80 + 16 * a + 32, :]
        r = lax.broadcasted_iota(jnp.int32, (32, 128), 0) + 16 * a
        return a, q, (r >= 20 * i) & (r < 20 * i + 20)

    def q_rows_shift(h, slot):
        g, i = h // 4, h % 4
        o_ = (20 * i) % 8
        q2 = QT[slot, g * 80 + 20 * i - o_: g * 80 + 20 * i - o_ + 24, :]
        r2 = lax.broadcasted_iota(jnp.int32, (24, 128), 0)
        c2 = lax.broadcasted_iota(jnp.int32, (24, 128), 1)
        return q2, (r2 >= o_) & (r2 < o_ + 20), c2

    def build_w(h, slot):
        a, q, rm = q_rows(h, slot)
        parts = []
        if a > 0:
            parts.append(jnp.zeros((16 * a, 128), f32))
        parts.append(jnp.where(rm, q, 0.0))
        parts.append(jnp.zeros((120 - 16 * a - 32, 128), f32))
        parts.append(jnp.where(sub8 == 7, 1.0, 0.0).astype(f32))
        return jnp.concatenate(parts, axis=0).astype(bf)

    def build_wd(h, slot):
        a, q, rm = q_rows(h, slot)
        c = lax.broadcasted_iota(jnp.int32, (32, 128), 1)
        q2, rm2, c2 = q_rows_shift(h, slot)
        parts = []
        if a > 0:
            parts.append(jnp.zeros((16 * a, 128), f32))
        parts.append(jnp.where(rm & (c < 64), q, 0.0))
        if 80 - 16 * a - 32 > 0:
            parts.append(jnp.zeros((80 - 16 * a - 32, 128), f32))
        parts.append(jnp.where(rm2 & (c2 >= 64), q2, 0.0))
        parts.append(jnp.zeros((16, 128), f32))
        parts.append(jnp.where((sub8 == 7) & (col8 < 64), 1.0, 0.0).astype(f32))
        return jnp.concatenate(parts, axis=0).astype(bf)

    def build_wd2(h, slot):
        q2, rm2, c2 = q_rows_shift(h, slot)
        parts = [jnp.where(rm2 & (c2 >= 32 * s_) & (c2 < 32 * s_ + 32), q2, 0.0) for s_ in range(4)]
        parts.append(jnp.zeros((24, 128), f32))
        parts.append(jnp.where((sub8 == 7) & ((col8 // 32) % 2 == 0), 1.0, 0.0).astype(f32))
        return jnp.concatenate(parts, axis=0).astype(bf)

    def qk_dot(b, h, slot, order):
        g, i = h // 4, h % 4
        lo, hi = g * 128, (g + 1) * 128
        o_ = (20 * i) % 8
        w = build_w(h, slot)
        kt = jnp.concatenate([KP[b + 2, 0:32, lo:hi], KP[b, 96:128, lo:hi], KP[b + 1, :, lo:hi]], axis=0)
        rl = pltpu.roll(KP[b + 2, 32:96, lo:hi], 80 + o_ - 20 * i, 1)
        ld = jnp.where((lane64 >= 80) & (lane64 < 104), rl, KP[b, 32:96, lo:hi])
        srcs = [KP[b, 0:32, lo:hi], KP[b + 2, 32:64, lo:hi], KP[b, 64:96, lo:hi], KP[b + 2, 96:128, lo:hi]]
        l2 = None
        for s_ in range(4):
            d_ = 24 * s_ + o_
            shift = (d_ - 20 * i) % 128
            v = pltpu.roll(srcs[s_], shift, 1) if shift else srcs[s_]
            if s_ == 0:
                l2 = jnp.where(lane32 == 127, srcs[0], v) if shift else v
            else:
                l2 = jnp.where((lane32 >= d_) & (lane32 < d_ + 20), v, l2)
        res = {}
        for ch in order:
            if ch == 'm':
                res[ch] = jnp.dot(kt, w, preferred_element_type=f32)
            elif ch == 'c':
                res[ch] = jnp.dot(ld, build_wd(h, slot), preferred_element_type=f32)
            else:
                res[ch] = jnp.dot(l2, build_wd2(h, slot), preferred_element_type=f32)
        return res['m'], res['c'], res['d']

    def max_stage(sd):
        si, cb, dg = sd
        mx = None
        scs = []
        for a in range(16):
            tri = sub8 + 8 * a > col8
            d_ = dg[8 * (a % 4):8 * (a % 4) + 8]
            if a < 4:
                sc = jnp.where(tri, d_, si[8 * a:8 * a + 8])
            elif a < 8:
                sc = jnp.where((col8 >= 32) & (col8 < 64) & jnp.logical_not(tri), d_, cb[8 * a - 32:8 * a - 24])
            elif a < 12:
                sc = jnp.where((col8 >= 64) & (col8 < 96) & tri, d_, cb[8 * a - 32:8 * a - 24])
            else:
                sc = jnp.where(tri, si[8 * a - 64:8 * a - 56], d_)
            scs.append(sc)
            mx = sc if mx is None else jnp.maximum(mx, sc)
        sm = si[64:192]
        for a in range(16):
            mx = jnp.maximum(mx, sm[8 * a:8 * a + 8])
        mx = jnp.max(mx, axis=0, keepdims=True)
        return (jnp.concatenate(scs, axis=0), sm, mx)

    def exp_pv(b, h, st):
        sc, sm, m = st
        row = lax.broadcasted_iota(jnp.int32, (128, 128), 0)
        pc = jnp.exp2(sc - m)
        pm = jnp.exp2(sm - m)
        msk = row > lane
        pu = jnp.where(msk, pc, 0.0)
        pl_ = jnp.where(msk, 0.0, pc)
        pall = jnp.concatenate([pu, pm, pl_], axis=0).astype(bf)
        vt = jnp.concatenate([VT[b + t, 32 * h:32 * h + 32, :] for t in range(3)], axis=1)
        o = jnp.dot(vt, pall, preferred_element_type=f32)
        l = o[20:21, :] if h % 2 == 0 else o[0:1, :]
        r = pltpu.reciprocal(l, approx=False)
        return o[0:24] * r

    def fin_o():
        for kt in range(5):
            OS[:, 128 * kt:128 * kt + 128] = OT[128 * kt:128 * kt + 128, :].T.astype(bf)

    def outproj(bprev):
        y = jnp.dot(OS[...], wo_v[...], preferred_element_type=f32)
        Y[1, pl.ds(pl.multiple_of(bprev * 128, 128), 128), :] = y.astype(bf)

    def out_copy(bb, half):
        rows = pl.ds(pl.multiple_of(bb * 128, 128), 128)
        return pltpu.make_async_copy(Y.at[half, rows, :],
                                     out_h.at[rows, pl.ds(pl.multiple_of(640 * half, 128), 640)], osem.at[0])

    units = [(a, j) for a in range(4) for j in range(4)]
    bsplit = [(0, 1, 2), (3, 4, 5), (6, 7)]

    def r5_fwd(u, bs):
        a, j = units[u]
        for b in bs:
            xs = [xa[a, b, 16 * j:16 * j + 16, 128 * t:128 * t + 128].astype(f32) for t in range(5)]
            o = _radix5_fwd(xs)
            for t in range(5):
                XL[u % 3, 16 * b:16 * b + 16, 128 * t:128 * t + 128] = o[t].astype(bf)

    def dfwd_dot(u, n):
        if n == 0:
            r_ = jnp.dot(XL[u % 3, :, 128:384], tb(g_v[0]), preferred_element_type=f32)
            return (r_[:, 0:128], r_[:, 128:256])
        if n == 1:
            r_ = jnp.dot(XL[u % 3, :, 384:640], tb(g_v[1]), preferred_element_type=f32)
            return (r_[:, 0:128], r_[:, 128:256])
        return jnp.dot(XL[u % 3, :, 0:128], tb(g_v[2, 0:64, 0:128]), preferred_element_type=f32)

    def fwd_fft_unit(a, p, j, t):
        for hh in range(2):
            xs = []
            for b in range(8):
                r = slice(16 * b + 8 * hh, 16 * b + 8 * hh + 8)
                if p < 2:
                    re = t[0][r]
                    im = t[1][r]
                else:
                    m = t[r]
                    re = jnp.where(col8 <= 64, m, 0.0)
                    im = jnp.where((col8 >= 1) & (col8 < 64), pltpu.roll(m, 64, 1), 0.0)
                xs.append((re, im))
            ys = _fft(xs, -1)
            rr = slice(16 * j + 8 * hh, 16 * j + 8 * hh + 8)
            for kp in range(8):
                y = _cmul_const(ys[kp], -2 * np.pi * a * kp / 32)
                PR[p, a * 8 + kp, rr, :] = y[0]
                PI[p, a * 8 + kp, rr, :] = y[1]

    def wretile(c):
        cs = slice(128 * (c % 8), 128 * (c % 8) + 128)
        WU[c, 0] = pltpu.bitcast(wr_v[c // 8, 0:320, cs], u32)
        WU[c, 1] = pltpu.bitcast(wi_v[c // 8, 0:320, cs], u32)

    def wprep1(c, p):
        def rows(rho):
            sl = pl.ds(rho // 2, 32, stride=5)
            a_ = upk(WU[c, 0, sl, :], rho % 2)
            b_ = upk(WU[c, 1, sl, :], rho % 2)
            if rho == 0:
                r32 = lax.broadcasted_iota(jnp.int32, (32, 128), 0)
                a_ = jnp.where(r32 == 0, 0.5 * a_, a_)
                b_ = jnp.where(r32 == 0, 0.5 * b_, b_)
            return (pltpu.bitcast(a_, u32) >> 16) | pltpu.bitcast(b_, u32)
        if p < 2:
            r1, r2 = (1, 4) if p == 0 else (2, 3)
            w = jnp.concatenate([rows(r1), rows(r1 + 5), rows(r2), rows(r2 + 5)], axis=0)
        else:
            cs = slice(128 * (c % 8), 128 * (c % 8) + 128)
            a_ = jnp.where(sub8 == 0, 0.5 * jnp.broadcast_to(wr_v[c // 8, 320:321, cs].astype(f32), (8, 128)), 0.0)
            b_ = jnp.where(sub8 == 0, 0.5 * jnp.broadcast_to(wi_v[c // 8, 320:321, cs].astype(f32), (8, 128)), 0.0)
            nyq = (pltpu.bitcast(a_, u32) >> 16) | pltpu.bitcast(b_, u32)
            w = jnp.concatenate([rows(0), rows(5), nyq, jnp.zeros((56, 128), u32)], axis=0)
        w = w.T
        for q in range(4):
            WW[p, pl.ds(33 * (4 * c + q), 32), :] = w[32 * q:32 * q + 32]

    def build_e():
        comp = lambda v: ((v % 16) // 8, 8 * (v // 16) + v % 8)
        pre_ = lambda v: 16 * (v // 16) + 2 * (v % 8) + (v % 16) // 8
        for blk in range(16):
            r = sub8 + 8 * blk
            for form in range(2):
                (cr, k2_), (cc, s2_) = (comp(pre_(r)), comp(col8)) if form == 0 else (comp(r), comp(pre_(col8)))
                th = ((k2_ * s2_) % 64).astype(f32) * float(2 * np.pi / 64)
                cs_, sn_ = jnp.cos(th), jnp.sin(th)
                same = cr == cc
                e_v[2 * form, 8 * blk:8 * blk + 8, :] = jnp.where(same, cs_, jnp.where(cr == 1, -sn_, sn_))
                e_v[2 * form + 1, 8 * blk:8 * blk + 8, :] = jnp.where(same, sn_, jnp.where(cr == 1, cs_, -cs_))

    def mbuild(k1):
        cf = jnp.broadcast_to(cs_v[0, k1:k1 + 1, :], (8, 128))
        sf = jnp.broadcast_to(cs_v[1, k1:k1 + 1, :], (8, 128))
        for v in range(8):
            lo = e_v[0, 16 * v:16 * v + 8, :] * cf + e_v[1, 16 * v:16 * v + 8, :] * sf
            hi = e_v[0, 16 * v + 8:16 * v + 16, :] * cf + e_v[1, 16 * v + 8:16 * v + 16, :] * sf
            mf_v[k1, 8 * v:8 * v + 8, :] = pk2(lo, hi)
        ci = jnp.broadcast_to(cs_v[2, k1:k1 + 1, :], (8, 128))
        si = jnp.broadcast_to(cs_v[3, k1:k1 + 1, :], (8, 128))
        nn = jnp.concatenate([e_v[2, 8 * r:8 * r + 8, :] * ci + e_v[3, 8 * r:8 * r + 8, :] * si
                              for r in range(16)], axis=0).T
        for v in range(8):
            mi_v[k1, 8 * v:8 * v + 8, :] = pk2(nn[16 * v:16 * v + 8], nn[16 * v + 8:16 * v + 16])

    def pre(kp, p):
        tl = [[] for _ in range(4)]
        for g in range(8):
            v = [(PR[p, a * 8 + kp, 8 * g:8 * g + 8, :], PI[p, a * 8 + kp, 8 * g:8 * g + 8, :]) for a in range(4)]
            ts = _radix4(v, -1)
            for kk in range(4):
                tl[kk] += [ts[kk][0], ts[kk][1]]
        return [jnp.concatenate(t_, axis=0).astype(bf) for t_ in tl]

    def fwd(kp, ts):
        return [jnp.dot(tb(mf_v[kp + 8 * kk]), ts[kk], preferred_element_type=f32) for kk in range(4)]

    def mid(u, kp, p, xs):
        for g in range(8):
            for kk in range(4):
                k1 = kp + 8 * kk
                x = xs[kk]
                xr, xi = x[16 * g:16 * g + 8], x[16 * g + 8:16 * g + 16]
                ww = WW[p, pl.ds(k1 + 33 * 8 * g, 8, stride=33), :]
                wr = upk(ww, 0)
                wi = upk(ww, 1)
                YS[u % 3, kk, 16 * g:16 * g + 16, :] = jnp.concatenate(
                    [xr * wr - xi * wi, xr * wi + xi * wr], axis=0).astype(bf)

    def inv(u, kp):
        return [jnp.dot(tb(mi_v[kp + 8 * kk]), YS[u % 3, kk], preferred_element_type=f32) for kk in range(4)]

    def post(kp, p, outs):
        for g in range(8):
            v = [(o[16 * g:16 * g + 8], o[16 * g + 8:16 * g + 16]) for o in outs]
            r = _radix4(v, +1)
            for a in range(4):
                PR[p, a * 8 + kp, 8 * g:8 * g + 8, :] = r[a][0]
                PI[p, a * 8 + kp, 8 * g:8 * g + 8, :] = r[a][1]

    def inv_unit_p(u, p):
        a, j = units[u]
        for hh in range(2):
            rr = slice(16 * j + 8 * hh, 16 * j + 8 * hh + 8)
            xs = []
            for kp in range(8):
                v = (PR[p, a * 8 + kp, rr, :], PI[p, a * 8 + kp, rr, :])
                xs.append(_cmul_const(v, 2 * np.pi * a * kp / 32))
            zs = _fft(xs, +1)
            for b in range(8):
                r = slice(16 * b + 8 * hh, 16 * b + 8 * hh + 8)
                zr, zi = zs[b]
                if p == 2:
                    ZF[u % 3, r, 0:128] = jnp.where(col8 <= 64, zr, pltpu.roll(zi, 64, 1))
                elif p == 0:
                    ZF[u % 3, r, 128:256] = zr
                    ZF[u % 3, r, 256:384] = zi
                else:
                    ZF[u % 3, r, 384:512] = zr
                    ZF[u % 3, r, 512:640] = zi

    def dinv_dot(u, n):
        if n == 0:
            return lax.dot_general(ZF[u % 3, :, 128:384].astype(bf), tb(g_v[0]), _NT, preferred_element_type=f32)
        if n == 1:
            return lax.dot_general(ZF[u % 3, :, 384:640].astype(bf), tb(g_v[1]), _NT, preferred_element_type=f32)
        return lax.dot_general(ZF[u % 3, :, 0:128].astype(bf), tb(g_v[2, 0:64, 0:128]), _NT, preferred_element_type=f32)

    def r5_inv(u, qs, bs):
        a, j = units[u]
        q1, q2, q0 = qs
        for b in bs:
            r = slice(16 * b, 16 * b + 16)
            ys = _radix5_inv(q0[r], q1[r, 0:128], q1[r, 128:256], q2[r, 0:128], q2[r, 128:256])
            for t in range(5):
                Y[0, pl.ds(64 * (a + 4 * b) + 16 * j, 16), 128 * t:128 * t + 128] = ys[t].astype(bf)

    def wt_job(i, half):
        base = 0 if half == 0 else 1280
        wT[640 * half + 128 * i:640 * half + 128 * i + 128, :] = wqkv_v[:, base + 128 * i:base + 128 * i + 128].T

    a_out = pltpu.make_async_copy(Y.at[0, pl.ds(128, S_ - 128), :],
                                  out_h.at[pl.ds(128, S_ - 128), pl.ds(0, 640)], osem.at[1])

    build_e()
    init_pads()
    cp_xa[0].wait()
    wjobs = [(c, p_) for c in range(16) for p_ in range(3)]
    r5_fwd(0, range(8))
    r5_fwd(1, range(8))
    cp_g.wait()
    cp_cs.wait()
    dres = {}
    for q in range(48 + 1):
        qq = q - 1
        if qq >= 0 and qq % 3 == 0:
            u = qq // 3
            if u + 2 < 16 and units[u + 2][1] == 0:
                cp_xa[units[u + 2][0]].wait()
            if u == 12:
                for c_ in cp_wg[0]:
                    c_.wait()
        if q < 48:
            dres[q] = dfwd_dot(q // 3, q % 3)
        if qq < 0:
            continue
        u, n = qq // 3, qq % 3
        if u + 2 < 16:
            r5_fwd(u + 2, bsplit[n])
        if 12 <= u < 16:
            k_ = (u - 12) * 3 + n
            if k_ == 0:
                for c_i in range(8):
                    wretile(c_i)
            for jb in wjobs[2 * k_:2 * k_ + 2]:
                wprep1(*jb)
        if 6 <= qq < 6 + R:
            mbuild(qq - 6)
        fwd_fft_unit(u // 4, n, u % 4, dres.pop(qq))
    for c_ in cp_wg[1]:
        c_.wait()
    for c_i in range(8, 16):
        wretile(c_i)
    for c_i in range(8, 16):
        wprep1(c_i, 0)
    us = [(kp, p) for p in range(3) for kp in range(8)]
    xr_ = {}
    or_ = {}
    tl_ = {0: pre(*us[0])}
    for t in range(24 + 3):
        if t < 24:
            xr_[t] = fwd(us[t][0], tl_.pop(t))
        if t >= 3:
            post(*us[t - 3], or_.pop(t - 3))
        if t + 1 < 24:
            tl_[t + 1] = pre(*us[t + 1])
        if 2 <= t < 26:
            or_[t - 2] = inv(t - 2, us[t - 2][0])
        if t < 16:
            wprep1(8 + t % 8, 1 + t // 8)
        if t < 24:
            mid(t, *us[t], xr_.pop(t))
    cp_w.wait()
    cp_xb[0].wait()
    x0 = xb[0:128, :]
    proj_k(0, x0)
    for p in range(3):
        inv_unit_p(0, p)
    for p in range(3):
        inv_unit_p(1, p)
    qres = {}
    for u in range(16 + 1):
        for n in range(3):
            if u < 16:
                qres[(u, n)] = dinv_dot(u, n)
            if u + 2 < 16:
                inv_unit_p(u + 2, n)
            if u >= 1:
                r5_inv(u - 1, [qres[(u - 1, 0)], qres[(u - 1, 1)], qres[(u - 1, 2)]], bsplit[n])
            if n == 2 and 1 <= u < 11:
                wt_job((u - 1) // 2, (u - 1) % 2)
        if u == 15:
            proj_qv(0, x0, 0)
    a_out.start()
    cp_wo.wait()
    cp_xb[1].wait()

    def step(b, last):
        slot = b % 2
        bp = b - 1 if last else jnp.maximum(b - 1, 0)
        order = 'dcm' if last else 'dmc'
        t_out = NH + 1 if last else 2
        dots = {}
        sts = {}
        outs = {}
        if not last:
            bn = b + 1
        for t in range(NH + LAG):
            if t < NH:
                dots[t] = qk_dot(b, t, slot, order)
            if t == 0:
                fin_o()
            if t == t_out:
                outproj(bp)
            if 0 <= t - 2 < NH:
                sts[t - 2] = max_stage(dots.pop(t - 2))
            if t == NH and not last:
                xn = xb[pl.ds(pl.multiple_of(bn * 128, 128), 128), :]
                proj_k(bn, xn)
            if 0 <= t - LAG < NH:
                h = t - LAG
                outs[h] = exp_pv(b, h, sts.pop(h))
                if h % 2 == 1:
                    A = outs.pop(h - 1)
                    B = outs.pop(h)
                    p = h // 2
                    OT[40 * p:40 * p + 40, :] = jnp.concatenate(
                        [A[0:16], jnp.where(sub8 < 4, A[16:24], B[0:8]), B[8:24]], axis=0)
        if last:
            out_copy(bp, 1).start()
        else:
            proj_qv(bn, xn, 1 - slot)
            out_copy(bp, jnp.minimum(b, 1)).start()

    def body(b, carry):
        step(b, False)
        return carry

    lax.fori_loop(0, NB - 1, body, 0, unroll=UNROLL)
    step(NB - 1, True)
    fin_o()
    lastc = []
    r0 = (NB - 1) * 128
    for n in range(5):
        y_ = jnp.dot(OS[...], wo_v[:, 128 * n:128 * n + 128], preferred_element_type=f32)
        Y[1, r0:r0 + 128, 128 * n:128 * n + 128] = y_.astype(bf)
        c_ = pltpu.make_async_copy(Y.at[1, pl.ds(r0, 128), pl.ds(128 * n, 128)],
                                   out_h.at[pl.ds(r0, 128), pl.ds(640 + 128 * n, 128)], osem.at[2])
        c_.start()
        lastc.append(c_)
    a_out.wait()
    for i in range(NB):
        out_copy(0, 1).wait()
    for c_ in lastc:
        c_.wait()


@jax.jit
def pallas_concat_heads__spectral_gfnet__sliding_block__prompt_kernel(
    A_x: jax.Array,
    A_w_r: jax.Array,
    A_w_i: jax.Array,
    B_x: jax.Array,
    B_wqkv: jax.Array,
    B_wo: jax.Array,
):
    hbm = pl.BlockSpec(memory_space=pltpu.HBM)
    V = pltpu.VMEM
    out = pl.pallas_call(
        _kernel,
        out_shape=jax.ShapeDtypeStruct((S_, 2 * D), bf),
        in_specs=[hbm] * 8,
        out_specs=hbm,
        scratch_shapes=[
            V((4, 8, 64, D), bf), V((2, 321, 1024), bf), V((2, 321, 1024), bf),
            V((3, 128, 256), u32), V((R, 64, 128), u32), V((R, 64, 128), u32),
            V((4, 128, 128), f32), V((4, R, 128), f32),
            V((3, 32, 64, 128), f32), V((3, 32, 64, 128), f32),
            V((3, 2112, 128), u32),
            V((2, S_, D), bf), V((3, 4, 128, 128), bf), V((3, 128, D), f32), V((3, 128, D), bf),
            V((16, 2, 160, 128), u32),
            V((S_, D), bf), V((D, 3 * D), bf), V((D, D), bf), V((2 * D, D), bf),
            V((NB + 2, 128, 1024), bf), V((NB + 2, 1024, 128), bf),
            V((2, D, 128), f32), V((D, 128), f32), V((128, D), bf),
            pltpu.SemaphoreType.DMA((10,)), pltpu.SemaphoreType.DMA((3,)),
        ],
        compiler_params=pltpu.CompilerParams(vmem_limit_bytes=110 * 2**20),
        name='fused',
    )(A_x.reshape(8, 4, 64, D), A_w_r.T, A_w_i.T, B_x.reshape(S_, D), B_wqkv, B_wo,
      jnp.asarray(G_U32), jnp.asarray(CS_NP))
    return out.reshape(1, S_, 2 * D)
```
